```python
import jax
import jax.numpy as jnp

def _softmax(x, axis=-1):
    return jax.nn.softmax(x, axis=axis)

def _gelu(x):
    return jax.nn.gelu(x, approximate=True)

def _silu(x):
    return jax.nn.silu(x)

def _sigmoid(x):
    return jax.nn.sigmoid(x)

def _layernorm(x, axis=-1, eps=1e-05):
    m = jnp.mean(x, axis=axis, keepdims=True)
    v = jnp.var(x, axis=axis, keepdims=True)
    return (x - m) / jnp.sqrt(v + eps)

def _scatter_add(tgt, idx, src, axis=0):
    return tgt.at[idx].add(src)

def _segment_sum(src, seg, n):
    return jax.ops.segment_sum(src, seg, n)

class _Rng:

    def __init__(self, key):
        self._k = key

    def _next(self):
        self._k, sub = jax.random.split(self._k)
        return sub

    def normal(self, shape):
        return jax.random.normal(self._next(), shape, dtype=jnp.bfloat16)

    def randint(self, lo, hi, shape):
        return jax.random.randint(self._next(), shape, lo, hi, dtype=jnp.int32)

    def uniform(self, shape, lo=0.0, hi=1.0):
        return jax.random.uniform(self._next(), shape, jnp.bfloat16, lo, hi)

    def permutation(self, n):
        return jax.random.permutation(self._next(), n)
kernel_name = 'adaLN_cond__gqa_block_cached__moe_arch_mod__prompt'

def setup_inputs():
    _rng = _Rng(jax.random.key(int.from_bytes(__import__("os").urandom(4), "little")))
    _w = lambda a: (lambda t: t.astype(jnp.bfloat16) if jnp.issubdtype(t.dtype, jnp.floating) else t)(jnp.asarray(a))

    def _A_setup():
        B, Sq, D = (1, 2048, 576)
        Hq, Hkv, Sk, Dh = (32, 16, 2048, 128)
        assert Hq % Hkv == 0, (Hq, Hkv)
        return {'x': _w((lambda *s: _rng.normal(s) * 0.05)(B, Sq, D)), 'k_cache': _w((lambda *s: _rng.normal(s) * 0.05)(B, Hkv, Sk, Dh)), 'v_cache': _w((lambda *s: _rng.normal(s) * 0.05)(B, Hkv, Sk, Dh)), 'wq': _w((lambda *s: _rng.normal(s) * 0.05)(D, Hq * Dh) * D ** (-0.5)), 'wo': _w((lambda *s: _rng.normal(s) * 0.05)(Hq * Dh, D) * (Hq * Dh) ** (-0.5))}
    _A_in = _A_setup()

    def _B_setup():
        B, S, D, F, C = (1, 2048, 576, 4608, 8)
        return {'x': _w((lambda *s: _rng.normal(s) * 0.05)(B, S, D)), 'w_r': _w((lambda *s: _rng.normal(s) * 0.05)(D)), 'w_gate': _w((lambda *s: _rng.normal(s) * 0.05)(D, F)), 'w_up': _w((lambda *s: _rng.normal(s) * 0.05)(D, F)), 'w_down': _w((lambda *s: _rng.normal(s) * 0.05)(F, D))}
    _B_in = _B_setup()
    return {'A_x': _A_in['x'], 'A_k_cache': _A_in['k_cache'], 'A_v_cache': _A_in['v_cache'], 'A_wq': _A_in['wq'], 'A_wo': _A_in['wo'], 'B_x': _B_in['x'], 'B_w_r': _B_in['w_r'], 'B_w_gate': _B_in['w_gate'], 'B_w_up': _B_in['w_up'], 'B_w_down': _B_in['w_down'], 'c': _w((lambda *s: _rng.normal(s) * 0.05)(1, 576)), 'w_mod': _w((lambda *s: _rng.normal(s) * 0.05)(576, 6 * 576) * 576 ** (-0.5))}

def reference(A_x, A_k_cache, A_v_cache, A_wq, A_wo, B_x, B_w_r, B_w_gate, B_w_up, B_w_down, c, w_mod):

    def _A_ref(x, k_cache, v_cache, wq, wo):
        B, Sq, D = x.shape
        Hq, Dh = (32, 128)
        Hkv = k_cache.shape[1]
        rep = Hq // Hkv
        q = (lambda x, *d: x.transpose(*d))((x @ wq).reshape(B, Sq, Hq, Dh), 0, 2, 1, 3)
        k = jnp.repeat(k_cache, rep, axis=1)
        v = jnp.repeat(v_cache, rep, axis=1)
        scores = jnp.einsum('bhqd,bhkd->bhqk', q, k) * Dh ** (-0.5)
        p = _softmax(scores, axis=-1)
        o = jnp.einsum('bhqk,bhkd->bhqd', p, v)
        return (lambda x, *d: x.transpose(*d))(o, 0, 2, 1, 3).reshape(B, Sq, Hq * Dh) @ wo

    def _B_ref(x, w_r, w_gate, w_up, w_down):
        B, S, D = x.shape
        C = 8
        r = x @ w_r
        idx = jnp.argsort(-r, axis=-1)[:, :C]
        idx_e = jnp.repeat(idx.reshape(B, C, 1), D, axis=2)
        x_sel = jnp.take_along_axis(x, idx_e, axis=1)
        g = _silu(x_sel @ w_gate)
        u = x_sel @ w_up
        y = g * u @ w_down
        r_sel = _sigmoid(jnp.take_along_axis(r, idx, axis=1))
        y = y * r_sel.reshape(B, C, 1)
        b_off = (jnp.arange(B) * S).reshape(B, 1)
        flat_idx = (idx + b_off).reshape(B * C)
        zero = (x * 0.0).reshape(B * S, D)
        upd = _scatter_add(zero, flat_idx, y.reshape(B * C, D), axis=0)
        return x + upd.reshape(B, S, D)
    x = A_x
    mod = (_silu(c) @ w_mod).reshape(c.shape[0], 6, 1, -1)
    sa, ca, ga, sb, cb, gb = (mod[:, 0].copy(), mod[:, 1].copy(), mod[:, 2].copy(), mod[:, 3].copy(), mod[:, 4].copy(), mod[:, 5].copy())
    h = _layernorm(x, axis=-1) * (1 + ca) + sa
    x = x + ga * _A_ref(h, A_k_cache, A_v_cache, A_wq, A_wo)
    h = _layernorm(x, axis=-1) * (1 + cb) + sb
    x = x + gb * _B_ref(h, B_w_r, B_w_gate, B_w_up, B_w_down)
    return x
```

```python
import functools

import jax
import jax.numpy as jnp
import jax.experimental.pallas as pl
import jax.experimental.pallas.tpu as pltpu
import numpy as np
from jax import lax

F32 = jnp.float32
BF16 = jnp.bfloat16
I32 = jnp.int32

NT_DIMS = (((1,), (1,)), ((), ()))
TOPC = 8
LN_EPS = 1e-5
LN_EPS_BF16 = float(np.asarray(LN_EPS, dtype=jnp.bfloat16))
LOG2E = 1.4426950408889634

RB = 256
BQ = 512
SPI = 2


def _rb(a):
    return a.astype(BF16).astype(F32)


def _pack(a):
    return pltpu.bitcast(a, I32)


def _unpack(a):
    return pltpu.bitcast(a, BF16)


def _fold(a, op):
    out = a[:, :128]
    for j in range(1, a.shape[1] // 128):
        out = op(out, a[:, j * 128:(j + 1) * 128])
    return out


def _kernel(c_ref, wr_ref, x_hbm, k_hbm, v_hbm, wq_hbm, wo_hbm, wg_hbm, wu_hbm, wd_hbm,
            wmod_hbm, o_hbm,
            x_s, k_s, v_s, wq_s, wo_s, wg_s, wu_s, wd_s, wmod_s,
            q_s, o_s, s_s, m_s, hb_s, a_s, col_s, x1r_s, h2r_s, r_s,
            sem_x, sem_wq, sem_k, sem_v, sem_w, sem_o,
            *, S, D, HQ, HKV, DH, F):
    nrb = S // RB
    nwq = sem_wq.shape[0]
    wq_cols = (HQ * DH) // nwq
    mod_a = 2 * D
    rep = HQ // HKV
    nbh = S // BQ
    nblk = HQ * nbh
    half = BQ // 2
    k_i = k_s.bitcast(I32)
    v_i = v_s.bitcast(I32)

    def x_copy(i):
        cols = pl.ds(pl.multiple_of(i * RB, RB), RB)
        return pltpu.make_async_copy(x_hbm.at[:, cols], x_s.at[:, cols], sem_x.at[i])

    def out_copy(t):
        cols = pl.ds(pl.multiple_of(t * 128, 128), 128)
        return pltpu.make_async_copy(x_s.at[:, cols], o_hbm.at[:, cols], sem_o.at[t])

    def wq_copy(j):
        cols = pl.ds(j * wq_cols, wq_cols)
        return pltpu.make_async_copy(wq_hbm.at[:, cols], wq_s.at[:, cols], sem_wq.at[j])

    def k_copy(h):
        return pltpu.make_async_copy(k_hbm.at[h], k_s.at[h], sem_k.at[h])

    def v_copy(h):
        return pltpu.make_async_copy(v_hbm.at[h], v_s.at[h], sem_v.at[h])

    moda_copy = pltpu.make_async_copy(
        wmod_hbm.at[:, pl.ds(0, mod_a)], wmod_s.at[:, pl.ds(0, mod_a)], sem_w.at[0])
    modb_copy = pltpu.make_async_copy(
        wmod_hbm.at[:, pl.ds(mod_a, 4 * D)], wmod_s.at[:, pl.ds(mod_a, 4 * D)], sem_w.at[1])
    wo_copy = pltpu.make_async_copy(wo_hbm, wo_s, sem_w.at[2])
    wg_copy = pltpu.make_async_copy(wg_hbm, wg_s, sem_w.at[3])
    wu_copy = pltpu.make_async_copy(wu_hbm, wu_s, sem_w.at[4])
    wd_copy = pltpu.make_async_copy(wd_hbm, wd_s, sem_w.at[5])

    moda_copy.start()
    x_copy(0).start()
    for j in range(nwq):
        wq_copy(j).start()
    for i in range(1, nrb):
        x_copy(i).start()

    cv = c_ref[...].astype(F32)
    sc = _rb(cv * _rb(jax.nn.sigmoid(cv)))
    sc = jnp.broadcast_to(sc, (16, D)).astype(BF16)

    moda_copy.wait()
    mod = _rb(jnp.dot(sc, wmod_s[:, 0:mod_a], preferred_element_type=F32))[0:8]
    sa = mod[:, 0:D]
    ca1 = _rb(1.0 + mod[:, D:2 * D])

    def ln1(i):
        xv = x_s[:, pl.ds(pl.multiple_of(i * RB, RB), RB)].T.astype(F32)
        mean = jnp.sum(xv, axis=-1, keepdims=True) * (1.0 / D)
        xc = xv - mean
        var = jnp.sum(xc * xc, axis=-1, keepdims=True) * (1.0 / D)
        hn = xc * lax.rsqrt(var + LN_EPS)
        return (hn * jnp.tile(ca1, (RB // 8, 1)) + jnp.tile(sa, (RB // 8, 1))).astype(BF16)

    qscale = (DH ** -0.5) * LOG2E

    def q_proj(i, hb, wait):
        for j in range(nwq):
            if wait:
                wq_copy(j).wait()
            q = jnp.dot(hb, wq_s[:, j * wq_cols:(j + 1) * wq_cols], preferred_element_type=F32)
            for u in range(wq_cols // DH):
                q_s[j * (wq_cols // DH) + u,
                    pl.ds(pl.multiple_of(i * (RB // 2), RB // 2), RB // 2), :] = _pack(
                        (q[:, u * DH:(u + 1) * DH] * qscale).astype(BF16))

    x_copy(0).wait()
    hb_s[...] = ln1(0)
    x_copy(1).wait()
    h1 = ln1(1)
    q_proj(0, hb_s[...], True)
    hb_s[...] = h1

    def p1_body(i, carry):
        for u in range(2):
            k_copy(2 * (i - 1) + u).start()
            v_copy(2 * (i - 1) + u).start()
        x_copy(i + 1).wait()
        hb = hb_s[...]
        hn = ln1(i + 1)
        q_proj(i, hb, False)
        hb_s[...] = hn
        return carry

    lax.fori_loop(1, nrb - 1, p1_body, 0)
    for h in range(2 * (nrb - 2), HKV):
        k_copy(h).start()
        v_copy(h).start()
    modb_copy.start()
    wo_copy.start()
    wg_copy.start()
    wu_copy.start()
    wd_copy.start()
    q_proj(nrb - 1, hb_s[...], False)

    def qk(b, slot):
        hq = b // nbh
        q = _unpack(q_s[hq, pl.ds(pl.multiple_of((b % nbh) * half, half), half), :])
        kk = _unpack(k_i[hq // rep])
        s = lax.dot_general(q, kk, NT_DIMS, preferred_element_type=F32)
        s_s[slot] = s
        m = jnp.max(_fold(s, jnp.maximum), axis=-1, keepdims=True)
        m_s[slot] = jnp.broadcast_to(m, (BQ, 128))

    def pv(b, slot):
        hq = b // nbh
        m = m_s[slot]
        p = jnp.exp2(s_s[slot] - jnp.tile(m, (1, S // 128)))
        l = jnp.sum(_fold(p, jnp.add), axis=-1, keepdims=True)
        acc = jnp.dot(p.astype(BF16), _unpack(v_i[hq // rep]), preferred_element_type=F32)
        o = (acc * (1.0 / l)).astype(BF16)
        o_s[hq, pl.ds(pl.multiple_of((b % nbh) * half, half), half), :] = _pack(o)

    blk_per_kv = rep * nbh
    it_per_kv = blk_per_kv // SPI

    k_copy(0).wait()
    qk(0, 0)

    def p2_body(j, carry):
        h = j // it_per_kv

        @pl.when(j % it_per_kv == 0)
        def _():
            v_copy(h).wait()
            k_copy(h + 1).wait()

        for u in range(SPI):
            b = j * SPI + u
            qk(b + 1, (u + 1) % 2)
            pv(b, u % 2)
        return carry

    n_it = nblk // SPI
    lax.fori_loop(0, n_it - it_per_kv, p2_body, 0)
    v_copy(HKV - 1).wait()

    def p2_last(j, carry):
        for u in range(SPI):
            b = j * SPI + u
            qk(b + 1, (u + 1) % 2)
            pv(b, u % 2)
        return carry

    lax.fori_loop(n_it - it_per_kv, n_it - 1, p2_last, 0)
    for u in range(SPI):
        b = nblk - SPI + u
        if u != SPI - 1:
            qk(b + 1, (u + 1) % 2)
        pv(b, u % 2)

    modb_copy.wait()
    mod2 = _rb(jnp.dot(sc, wmod_s[:, mod_a:6 * D], preferred_element_type=F32))[0:8]
    gb = mod2[:, 3 * D:4 * D]
    for n, row in enumerate((mod2[:, 0:D], mod2[:, D:2 * D], _rb(1.0 + mod2[:, 2 * D:3 * D]), gb)):
        col_s[n] = jnp.broadcast_to(row[0:1], (128, D)).T
    wr = jnp.broadcast_to(wr_ref[...], (16, D))
    lanes = lambda a: jnp.tile(a, (1, RB // 128))

    def o_proj(i):
        rows = pl.ds(pl.multiple_of(i * (RB // 2), RB // 2), RB // 2)
        ob = jnp.concatenate([_unpack(o_s[h, rows, :]) for h in range(HQ)], axis=-1)
        return lax.dot_general(wo_s[...], ob, NT_DIMS, preferred_element_type=F32)

    def resid_norm(i, a):
        cols = pl.ds(pl.multiple_of(i * RB, RB), RB)
        rows = pl.ds(pl.multiple_of(i * (RB // 2), RB // 2), RB // 2)
        x1 = _rb(x_s[:, cols].astype(F32) + _rb(lanes(col_s[0]) * _rb(a)))
        mean = jnp.sum(x1, axis=0, keepdims=True) * (1.0 / D)
        xc = x1 - mean
        var = jnp.sum(xc * xc, axis=0, keepdims=True) * (1.0 / D)
        std = _rb(jnp.sqrt(_rb(_rb(var) + LN_EPS_BF16)))
        hn = _rb(_rb(x1 - _rb(mean)) / std)
        h2 = _rb(_rb(hn * lanes(col_s[2])) + lanes(col_s[1]))
        h2b = h2.astype(BF16)
        x1r_s[rows, :] = _pack(x1.astype(BF16).T)
        h2r_s[rows, :] = _pack(h2b.T)
        x_s[:, cols] = (x1 + _rb(lanes(col_s[3]) * h2)).astype(BF16)
        r = jnp.dot(wr, h2b, preferred_element_type=F32)
        r_s[:, cols] = _rb(r[0:8])
        for u in range(RB // 128):
            out_copy(i * (RB // 128) + u).start()

    wo_copy.wait()
    a_s[...] = o_proj(0)

    def p3_body(i, carry):
        a = a_s[...]
        an = o_proj(i + 1)
        resid_norm(i, a)
        a_s[...] = an
        return carry

    lax.fori_loop(0, nrb - 1, p3_body, 0)
    resid_norm(nrb - 1, a_s[...])

    r = r_s[...]
    col = lax.broadcasted_iota(I32, (8, S), 1)
    rbits = pltpu.bitcast(r, I32)
    key = pltpu.bitcast(rbits | jnp.where(rbits >= 0, (S - 1) - col, col), F32)
    sub = lax.broadcasted_iota(I32, (8, 128), 0)
    keyc = []
    for g in range(S // 1024):
        kc = key[:, g * 1024:g * 1024 + 128]
        for u in range(1, 8):
            kc = jnp.where(sub == u, key[:, g * 1024 + u * 128:g * 1024 + (u + 1) * 128], kc)
        keyc.append(kc)

    def token_row(ref, idx):
        word = ref[pl.ds(idx // 2, 1), :]
        bits = jnp.where(idx % 2 == 0, word << 16, word & jnp.int32(-65536))
        return pltpu.bitcast(jnp.broadcast_to(bits, (8, D)), F32)

    sub_d = lax.broadcasted_iota(I32, (8, D), 0)
    xsel = jnp.zeros((8, D), F32)
    x1sel = jnp.zeros((8, D), F32)
    best = jnp.zeros((8, 128), F32)
    idxs = []
    for j in range(TOPC):
        mx = functools.reduce(jnp.maximum, keyc)
        mx = jnp.max(jnp.max(mx, axis=0, keepdims=True), axis=1, keepdims=True)
        mxb = jnp.broadcast_to(mx, (8, 128))
        keyc = [jnp.where(kc == mxb, -jnp.inf, kc) for kc in keyc]
        best = jnp.where(sub == j, mxb, best)
        mb = pltpu.bitcast(mxb, I32)
        low = mb & (S - 1)
        idx = jnp.max(jnp.where(mb >= 0, (S - 1) - low, low))
        idxs.append(idx)
        xsel = jnp.where(sub_d == j, token_row(h2r_s, idx), xsel)
        x1sel = jnp.where(sub_d == j, token_row(x1r_s, idx), x1sel)

    rsel = pltpu.bitcast(pltpu.bitcast(best, I32) & jnp.int32(-65536), F32)[:, 0:1]
    xs = jnp.concatenate([xsel, xsel], axis=0).astype(BF16)
    wg_copy.wait()
    g = _rb(jnp.dot(xs, wg_s[...], preferred_element_type=F32)[0:8])
    wu_copy.wait()
    up = _rb(jnp.dot(xs, wu_s[...], preferred_element_type=F32)[0:8])
    act = _rb(_rb(g * _rb(jax.nn.sigmoid(g))) * up)
    act = jnp.concatenate([act, act], axis=0).astype(BF16)
    wd_copy.wait()
    y = _rb(lax.dot_general(act, wd_s[...], NT_DIMS, preferred_element_type=F32)[0:8])
    y = _rb(y * _rb(jax.nn.sigmoid(rsel)))
    new = _rb(x1sel + _rb(gb * _rb(xsel + y)))

    newc = _pack(jnp.concatenate([new, jnp.zeros((120, D), F32)], axis=0).astype(BF16).T)
    for t in range(S // 128):
        out_copy(t).wait()
    lane = lax.broadcasted_iota(I32, newc.shape, 1)
    x_i = x_s.bitcast(I32)
    for j in range(TOPC):
        cols = pl.ds(pl.multiple_of((idxs[j] // 128) * 128, 128), 128)
        moved = pltpu.roll(newc, (idxs[j] - j) % 128, 1)
        x_i[:, cols] = jnp.where(lane == idxs[j] % 128, moved, x_i[:, cols])

    tiles = [idx // 128 for idx in idxs]
    hits = [functools.reduce(jnp.logical_or, [tl == t for tl in tiles]) for t in range(S // 128)]
    for t in range(S // 128):
        @pl.when(hits[t])
        def _():
            out_copy(t).start()
    for t in range(S // 128):
        @pl.when(hits[t])
        def _():
            out_copy(t).wait()


@jax.jit
def pallas_adaLN_cond__gqa_block_cached__moe_arch_mod__prompt_kernel(
    A_x: jax.Array,
    A_k_cache: jax.Array,
    A_v_cache: jax.Array,
    A_wq: jax.Array,
    A_wo: jax.Array,
    B_x: jax.Array,
    B_w_r: jax.Array,
    B_w_gate: jax.Array,
    B_w_up: jax.Array,
    B_w_down: jax.Array,
    c: jax.Array,
    w_mod: jax.Array,
):
    del B_x
    B, S, D = A_x.shape
    _, HKV, SK, DH = A_k_cache.shape
    HQ = A_wq.shape[1] // DH
    F = B_w_gate.shape[1]
    assert B == 1 and SK == S and DH == 128 and S % 1024 == 0 and S <= 65536
    nwq = 8

    vm = pltpu.VMEM
    dma = pltpu.SemaphoreType.DMA
    hbm = pl.BlockSpec(memory_space=pl.ANY)
    small = pl.BlockSpec(memory_space=pltpu.VMEM)
    out = pl.pallas_call(
        functools.partial(_kernel, S=S, D=D, HQ=HQ, HKV=HKV, DH=DH, F=F),
        out_shape=jax.ShapeDtypeStruct((D, S), BF16),
        in_specs=[small, small] + [hbm] * 9,
        out_specs=hbm,
        scratch_shapes=[
            vm((D, S), BF16),
            vm((HKV, S, DH), BF16),
            vm((HKV, S, DH), BF16),
            vm((D, HQ * DH), BF16),
            vm((D, HQ * DH), BF16),
            vm((D, F), BF16),
            vm((D, F), BF16),
            vm((D, F), BF16),
            vm((D, 6 * D), BF16),
            vm((HQ, S // 2, DH), I32),
            vm((HQ, S // 2, DH), I32),
            vm((2, BQ, S), F32),
            vm((2, BQ, 128), F32),
            vm((RB, D), BF16),
            vm((D, RB), F32),
            vm((4, D, 128), F32),
            vm((S // 2, D), I32),
            vm((S // 2, D), I32),
            vm((8, S), F32),
            dma((S // RB,)), dma((nwq,)), dma((HKV,)), dma((HKV,)), dma((6,)), dma((S // 128,)),
        ],
        compiler_params=pltpu.CompilerParams(
            vmem_limit_bytes=118 * 1024 * 1024,
            flags={"XLA_TPU_FORCE_LP_LLO_SCHEDULER": True},
        ),
        name="adaln_gqa_moe_block",
    )(c, B_w_r.reshape(1, D), A_x[0].T, A_k_cache[0], A_v_cache[0], A_wq, A_wo.T,
      B_w_gate, B_w_up, B_w_down.T, w_mod)
    return out.T[None]
```

```python
import functools

import jax
import jax.numpy as jnp
import jax.experimental.pallas as pl
import jax.experimental.pallas.tpu as pltpu
import numpy as np
from jax import lax

F32 = jnp.float32
BF16 = jnp.bfloat16
I32 = jnp.int32

NT_DIMS = (((1,), (1,)), ((), ()))
TOPC = 8
LN_EPS = 1e-5
LN_EPS_BF16 = float(np.asarray(LN_EPS, dtype=jnp.bfloat16))
LOG2E = 1.4426950408889634

RB = 256
BQ = 1024
SPI = 2


def _rb(a):
    return a.astype(BF16).astype(F32)


def _pack(a):
    return pltpu.bitcast(a, I32)


def _unpack(a):
    return pltpu.bitcast(a, BF16)


def _fold(a, op):
    out = a[:, :128]
    for j in range(1, a.shape[1] // 128):
        out = op(out, a[:, j * 128:(j + 1) * 128])
    return out


def _kernel(c_ref, wr_ref, x_hbm, k_hbm, v_hbm, wq_hbm, wo_hbm, wg_hbm, wu_hbm, wd_hbm,
            wmod_hbm, o_hbm,
            x_s, k_s, v_s, wq_s, wo_s, wg_s, wu_s, wd_s, wmod_s,
            q_s, o_s, s_s, m_s, hb_s, a_s, col_s, x1r_s, h2r_s, r_s,
            sem_x, sem_wq, sem_k, sem_v, sem_w, sem_o,
            *, S, D, HQ, HKV, DH, F):
    nrb = S // RB
    nwq = sem_wq.shape[0]
    wq_cols = (HQ * DH) // nwq
    mod_a = 2 * D
    rep = HQ // HKV
    nbh = S // BQ
    nblk = HQ * nbh
    half = BQ // 2
    k_i = k_s.bitcast(I32)
    v_i = v_s.bitcast(I32)
    q_i = q_s.bitcast(I32)
    o_i = o_s.bitcast(I32)

    def x_copy(i):
        cols = pl.ds(pl.multiple_of(i * RB, RB), RB)
        return pltpu.make_async_copy(x_hbm.at[:, cols], x_s.at[:, cols], sem_x.at[i])

    def out_copy(t):
        cols = pl.ds(pl.multiple_of(t * 128, 128), 128)
        return pltpu.make_async_copy(x_s.at[:, cols], o_hbm.at[:, cols], sem_o.at[t])

    def wq_copy(j):
        cols = pl.ds(j * wq_cols, wq_cols)
        return pltpu.make_async_copy(wq_hbm.at[:, cols], wq_s.at[:, cols], sem_wq.at[j])

    def k_copy(h):
        return pltpu.make_async_copy(k_hbm.at[h], k_s.at[h], sem_k.at[h])

    def v_copy(h):
        return pltpu.make_async_copy(v_hbm.at[h], v_s.at[h], sem_v.at[h])

    moda_copy = pltpu.make_async_copy(
        wmod_hbm.at[:, pl.ds(0, mod_a)], wmod_s.at[:, pl.ds(0, mod_a)], sem_w.at[0])
    modb_copy = pltpu.make_async_copy(
        wmod_hbm.at[:, pl.ds(mod_a, 4 * D)], wmod_s.at[:, pl.ds(mod_a, 4 * D)], sem_w.at[1])
    wo_copy = pltpu.make_async_copy(wo_hbm, wo_s, sem_w.at[2])
    wg_copy = pltpu.make_async_copy(wg_hbm, wg_s, sem_w.at[3])
    wu_copy = pltpu.make_async_copy(wu_hbm, wu_s, sem_w.at[4])
    wd_copy = pltpu.make_async_copy(wd_hbm, wd_s, sem_w.at[5])

    moda_copy.start()
    x_copy(0).start()
    wq_copy(0).start()

    cv = c_ref[...].astype(F32)
    sc = _rb(cv * _rb(jax.nn.sigmoid(cv)))
    sc = jnp.broadcast_to(sc, (16, D)).astype(BF16)

    moda_copy.wait()
    wq_copy(1).start()
    x_copy(1).start()
    mod = _rb(jnp.dot(sc, wmod_s[:, 0:mod_a], preferred_element_type=F32))[0:8]
    sa = mod[:, 0:D]
    ca1 = _rb(1.0 + mod[:, D:2 * D])

    def ln1(i):
        xv = x_s[:, pl.ds(pl.multiple_of(i * RB, RB), RB)].T.astype(F32)
        mean = jnp.sum(xv, axis=-1, keepdims=True) * (1.0 / D)
        xc = xv - mean
        var = jnp.sum(xc * xc, axis=-1, keepdims=True) * (1.0 / D)
        hn = xc * lax.rsqrt(var + LN_EPS)
        return (hn * jnp.tile(ca1, (RB // 8, 1)) + jnp.tile(sa, (RB // 8, 1))).astype(BF16)

    qscale = (DH ** -0.5) * LOG2E

    npan = -(-D // 128)

    def put_h(slot, hn):
        for p in range(npan):
            w = min(128, D - p * 128)
            hb_s[slot, p, :, 0:w] = hn[:, p * 128:p * 128 + w]

    def get_h(slot):
        hb_i = hb_s.bitcast(I32)
        pans = [_unpack(hb_i[slot, p]) for p in range(npan)]
        return jnp.concatenate(pans, axis=-1)[:, 0:D]

    def q_proj(i, slot, wait, mid=None):
        for j in range(nwq):
            hb = get_h(slot)
            if mid is not None and j == 2:
                mid()
            if wait:
                wq_copy(j).wait()
                if j + 2 < nwq:
                    wq_copy(j + 2).start()
                if j == nwq - 1:
                    for ii in range(2, nrb):
                        x_copy(ii).start()
            q = jnp.dot(hb, wq_s[:, j * wq_cols:(j + 1) * wq_cols], preferred_element_type=F32)
            for u in range(wq_cols // DH):
                q_s[j * (wq_cols // DH) + u, pl.ds(pl.multiple_of(i * RB, RB), RB), :] = (
                    q[:, u * DH:(u + 1) * DH] * qscale).astype(BF16)

    x_copy(0).wait()
    hb_s[...] = jnp.zeros(hb_s.shape, BF16)
    put_h(0, ln1(0))
    x_copy(1).wait()
    h1 = ln1(1)
    q_proj(0, 0, True)
    put_h(1, h1)

    def p1_body(i, carry):
        def kv_start():
            for u in range(2):
                k_copy(2 * (i - 1) + u).start()
                v_copy(2 * (i - 1) + u).start()

        x_copy(i + 1).wait()
        hn = ln1(i + 1)
        q_proj(i, i & 1, False, kv_start)
        put_h((i + 1) & 1, hn)
        return carry

    lax.fori_loop(1, nrb - 1, p1_body, 0)

    def rest_start():
        for h in range(2 * (nrb - 2), HKV):
            k_copy(h).start()
            v_copy(h).start()
        for cp in (modb_copy, wo_copy, wg_copy, wu_copy, wd_copy):
            cp.start()

    q_proj(nrb - 1, (nrb - 1) & 1, False, rest_start)

    lg_kv = (rep * nbh).bit_length() - 1
    assert rep * nbh == 1 << lg_kv

    lg_h = nbh.bit_length() - 1
    assert nbh == 1 << lg_h

    def blk(b, size):
        return (lax.shift_right_logical(b, lg_h),
                pl.ds(pl.multiple_of((b & (nbh - 1)) * size, size), size))

    def finish_max(slot):
        m = jnp.max(m_s[slot], axis=-1, keepdims=True)
        m_s[slot] = jnp.broadcast_to(m, (BQ, 128))

    def qk(b, slot):
        q = _unpack(q_i[(*blk(b, half), slice(None))])
        kk = _unpack(k_i[lax.shift_right_logical(b, lg_kv)])
        s = lax.dot_general(q, kk, NT_DIMS, preferred_element_type=F32)
        s_s[slot] = s
        m_s[slot] = _fold(s, jnp.maximum)
        if slot == 0:
            finish_max(0)

    def pv(b, slot):
        m = m_s[slot]
        p = jnp.exp2(s_s[slot] - jnp.tile(m, (1, S // 128)))
        l = jnp.sum(_fold(p, jnp.add), axis=-1, keepdims=True)
        vv = _unpack(v_i[lax.shift_right_logical(b, lg_kv)])
        acc = jnp.dot(p.astype(BF16), vv, preferred_element_type=F32)
        inv = pl.reciprocal(l, approx=True)
        inv = inv * (2.0 - l * inv)
        o_s[(*blk(b, BQ), slice(None))] = (acc * inv).astype(BF16)

    it_per_kv = (rep * nbh) // SPI
    n_it = nblk // SPI

    k_copy(0).wait()
    qk(jnp.int32(0), 0)
    qk(jnp.int32(1), 1)

    def p2_steps(j, last):
        finish_max(1)
        for u in range(SPI):
            b = j * SPI + u
            pv(b, u % 2)
            if not (last and u >= SPI - 2):
                qk(b + 2, u % 2)

    def p2_body(j, carry):
        h = lax.shift_right_logical(j * SPI, lg_kv)

        @pl.when((j & (it_per_kv - 1)) == 0)
        def _():
            v_copy(h).wait()
            k_copy(h + 1).wait()

        p2_steps(j, False)
        return carry

    lax.fori_loop(0, n_it - it_per_kv, p2_body, 0)
    v_copy(HKV - 1).wait()

    def p2_last(j, carry):
        p2_steps(j, False)
        return carry

    lax.fori_loop(n_it - it_per_kv, n_it - 1, p2_last, 0)
    p2_steps(jnp.int32(n_it - 1), True)

    modb_copy.wait()
    mod2 = _rb(jnp.dot(sc, wmod_s[:, mod_a:6 * D], preferred_element_type=F32))[0:8]
    gb = mod2[:, 3 * D:4 * D]
    for n, row in enumerate((mod2[:, 0:D], mod2[:, D:2 * D], _rb(1.0 + mod2[:, 2 * D:3 * D]), gb)):
        col_s[n] = jnp.broadcast_to(row[0:1], (128, D)).T
    wr = jnp.broadcast_to(wr_ref[...], (16, D))
    lanes = lambda a: jnp.tile(a, (1, RB // 128))

    def o_proj(i):
        rows = pl.ds(pl.multiple_of(i * (RB // 2), RB // 2), RB // 2)
        ob = jnp.concatenate([_unpack(o_i[h, rows, :]) for h in range(HQ)], axis=-1)
        return lax.dot_general(wo_s[...], ob, NT_DIMS, preferred_element_type=F32)

    def resid_norm(i, a):
        cols = pl.ds(pl.multiple_of(i * RB, RB), RB)
        rows = pl.ds(pl.multiple_of(i * RB, RB), RB)
        x1 = _rb(x_s[:, cols].astype(F32) + _rb(lanes(col_s[0]) * _rb(a)))
        mean = jnp.sum(x1, axis=0, keepdims=True) * (1.0 / D)
        xc = x1 - mean
        var = jnp.sum(xc * xc, axis=0, keepdims=True) * (1.0 / D)
        std = _rb(jnp.sqrt(_rb(_rb(var) + LN_EPS_BF16)))
        hn = _rb(_rb(x1 - _rb(mean)) / std)
        h2 = _rb(_rb(hn * lanes(col_s[2])) + lanes(col_s[1]))
        h2b = h2.astype(BF16)
        x1r_s[rows, :] = x1.astype(BF16).T
        h2r_s[rows, :] = h2b.T
        x_s[:, cols] = (x1 + _rb(lanes(col_s[3]) * h2)).astype(BF16)
        r = jnp.dot(wr, h2b, preferred_element_type=F32)
        r_s[:, cols] = _rb(r[0:8])
        for u in range(RB // 128):
            out_copy(i * (RB // 128) + u).start()

    wo_copy.wait()
    a_s[...] = o_proj(0)

    def p3_body(i, carry):
        a = a_s[...]
        an = o_proj(i + 1)
        resid_norm(i, a)
        a_s[...] = an
        return carry

    lax.fori_loop(0, nrb - 1, p3_body, 0)
    resid_norm(nrb - 1, a_s[...])

    r = r_s[...]
    col = lax.broadcasted_iota(I32, (8, S), 1)
    rbits = pltpu.bitcast(r, I32)
    key = pltpu.bitcast(rbits | jnp.where(rbits >= 0, (S - 1) - col, col), F32)
    sub = lax.broadcasted_iota(I32, (8, 128), 0)
    keyc = []
    for g in range(S // 1024):
        kc = key[:, g * 1024:g * 1024 + 128]
        for u in range(1, 8):
            kc = jnp.where(sub == u, key[:, g * 1024 + u * 128:g * 1024 + (u + 1) * 128], kc)
        keyc.append(kc)

    def token_row(ref, idx):
        word = ref[pl.ds(idx // 2, 1), :]
        bits = jnp.where(idx % 2 == 0, word << 16, word & jnp.int32(-65536))
        return pltpu.bitcast(jnp.broadcast_to(bits, (8, D)), F32)

    sub_d = lax.broadcasted_iota(I32, (8, D), 0)
    xsel = jnp.zeros((8, D), F32)
    x1sel = jnp.zeros((8, D), F32)
    best = jnp.zeros((8, 128), F32)
    idxs = []
    for j in range(TOPC):
        mx = functools.reduce(jnp.maximum, keyc)
        mx = jnp.max(jnp.max(mx, axis=0, keepdims=True), axis=1, keepdims=True)
        mxb = jnp.broadcast_to(mx, (8, 128))
        keyc = [jnp.where(kc == mxb, -jnp.inf, kc) for kc in keyc]
        best = jnp.where(sub == j, mxb, best)
        mb = pltpu.bitcast(mxb, I32)
        low = mb & (S - 1)
        idx = jnp.max(jnp.where(mb >= 0, (S - 1) - low, low))
        idxs.append(idx)
        xsel = jnp.where(sub_d == j, token_row(h2r_s.bitcast(I32), idx), xsel)
        x1sel = jnp.where(sub_d == j, token_row(x1r_s.bitcast(I32), idx), x1sel)

    rsel = pltpu.bitcast(pltpu.bitcast(best, I32) & jnp.int32(-65536), F32)[:, 0:1]
    xs = jnp.concatenate([xsel, xsel], axis=0).astype(BF16)
    wg_copy.wait()
    g = _rb(jnp.dot(xs, wg_s[...], preferred_element_type=F32)[0:8])
    wu_copy.wait()
    up = _rb(jnp.dot(xs, wu_s[...], preferred_element_type=F32)[0:8])
    act = _rb(_rb(g * _rb(jax.nn.sigmoid(g))) * up)
    act = jnp.concatenate([act, act], axis=0).astype(BF16)
    wd_copy.wait()
    y = _rb(lax.dot_general(act, wd_s[...], NT_DIMS, preferred_element_type=F32)[0:8])
    y = _rb(y * _rb(jax.nn.sigmoid(rsel)))
    new = _rb(x1sel + _rb(gb * _rb(xsel + y)))

    newc = _pack(jnp.concatenate([new, jnp.zeros((120, D), F32)], axis=0).astype(BF16).T)
    for t in range(S // 128):
        out_copy(t).wait()
    lane = lax.broadcasted_iota(I32, newc.shape, 1)
    x_i = x_s.bitcast(I32)
    for j in range(TOPC):
        cols = pl.ds(pl.multiple_of((idxs[j] // 128) * 128, 128), 128)
        moved = pltpu.roll(newc, (idxs[j] - j) % 128, 1)
        x_i[:, cols] = jnp.where(lane == idxs[j] % 128, moved, x_i[:, cols])

    tiles = [idx // 128 for idx in idxs]
    hits = [functools.reduce(jnp.logical_or, [tl == t for tl in tiles]) for t in range(S // 128)]
    for t in range(S // 128):
        @pl.when(hits[t])
        def _():
            out_copy(t).start()
    for t in range(S // 128):
        @pl.when(hits[t])
        def _():
            out_copy(t).wait()


@jax.jit
def pallas_adaLN_cond__gqa_block_cached__moe_arch_mod__prompt_kernel(
    A_x: jax.Array,
    A_k_cache: jax.Array,
    A_v_cache: jax.Array,
    A_wq: jax.Array,
    A_wo: jax.Array,
    B_x: jax.Array,
    B_w_r: jax.Array,
    B_w_gate: jax.Array,
    B_w_up: jax.Array,
    B_w_down: jax.Array,
    c: jax.Array,
    w_mod: jax.Array,
):
    del B_x
    B, S, D = A_x.shape
    _, HKV, SK, DH = A_k_cache.shape
    HQ = A_wq.shape[1] // DH
    F = B_w_gate.shape[1]
    assert B == 1 and SK == S and DH == 128 and S % 1024 == 0 and S <= 65536
    nwq = 8

    vm = pltpu.VMEM
    dma = pltpu.SemaphoreType.DMA
    hbm = pl.BlockSpec(memory_space=pl.ANY)
    small = pl.BlockSpec(memory_space=pltpu.VMEM)
    out = pl.pallas_call(
        functools.partial(_kernel, S=S, D=D, HQ=HQ, HKV=HKV, DH=DH, F=F),
        out_shape=jax.ShapeDtypeStruct((D, S), BF16),
        in_specs=[small, small] + [hbm] * 9,
        out_specs=hbm,
        scratch_shapes=[
            vm((D, S), BF16),
            vm((HKV, S, DH), BF16),
            vm((HKV, S, DH), BF16),
            vm((D, HQ * DH), BF16),
            vm((D, HQ * DH), BF16),
            vm((D, F), BF16),
            vm((D, F), BF16),
            vm((D, F), BF16),
            vm((D, 6 * D), BF16),
            vm((HQ, S, DH), BF16),
            vm((HQ, S, DH), BF16),
            vm((2, BQ, S), F32),
            vm((2, BQ, 128), F32),
            vm((2, -(-D // 128), RB, 128), BF16),
            vm((D, RB), F32),
            vm((4, D, 128), F32),
            vm((S, D), BF16),
            vm((S, D), BF16),
            vm((8, S), F32),
            dma((S // RB,)), dma((nwq,)), dma((HKV,)), dma((HKV,)), dma((6,)), dma((S // 128,)),
        ],
        compiler_params=pltpu.CompilerParams(
            vmem_limit_bytes=118 * 1024 * 1024,
            flags={"XLA_TPU_FORCE_LP_LLO_SCHEDULER": True},
        ),
        name="adaln_gqa_moe_block",
    )(c, B_w_r.reshape(1, D), A_x[0].T, A_k_cache[0], A_v_cache[0], A_wq, A_wo.T,
      B_w_gate, B_w_up, B_w_down.T, w_mod)
    return out.T[None]
```

```python
import functools

import jax
import jax.numpy as jnp
import jax.experimental.pallas as pl
import jax.experimental.pallas.tpu as pltpu
import numpy as np
from jax import lax

F32 = jnp.float32
BF16 = jnp.bfloat16
I32 = jnp.int32

NT_DIMS = (((1,), (1,)), ((), ()))
TOPC = 8
LN_EPS = 1e-5
LN_EPS_BF16 = float(np.asarray(LN_EPS, dtype=jnp.bfloat16))
LOG2E = 1.4426950408889634

RB = 512
BQ = 512
TB = 256
WQ_CHUNK = 512
WQ_GROUPS = (1, 2, 4, 1)


def _rb(a):
    return a.astype(BF16).astype(F32)


def _unpack(a):
    return pltpu.bitcast(a, BF16)


def _fold(a, op):
    out = a[:, :128]
    for j in range(1, a.shape[1] // 128):
        out = op(out, a[:, j * 128:(j + 1) * 128])
    return out


def _kernel(c_ref, wr_ref, x_hbm, k_hbm, v_hbm, wq_hbm, wo_hbm, wg_hbm, wu_hbm, wd_hbm,
            wmod_hbm, o_hbm,
            x_s, k_s, v_s, wq_s, wo_s, wg_s, wu_s, wd_s, wmod_s,
            q_s, o_s, s_s, m_s, h_s, xn_s, a_s, col_s, h2r_s, r_s,
            sem_x, sem_wq, sem_w, sem_o, sem_f,
            *, S, D, HQ, HKV, DH):
    mod_a = 2 * D
    rep = HQ // HKV
    k_i = k_s.bitcast(I32)
    v_i = v_s.bitcast(I32)
    q_i = q_s.bitcast(I32)
    o_i = o_s.bitcast(I32)
    h_i = h_s.bitcast(I32)
    wo_i = wo_s.bitcast(I32)

    nrb = S // RB
    nwq = HQ * DH // WQ_CHUNK
    assert sum(WQ_GROUPS) == nwq and nrb >= 3
    g_lo = np.cumsum((0,) + WQ_GROUPS)

    def x_copy(g):
        cols = pl.ds(g * RB, RB if g < 2 else S - 2 * RB)
        return pltpu.make_async_copy(x_hbm.at[:, cols], x_s.at[:, cols], sem_x.at[g])

    def wq_copy(g):
        cols = pl.ds(int(g_lo[g]) * WQ_CHUNK, WQ_GROUPS[g] * WQ_CHUNK)
        return pltpu.make_async_copy(wq_hbm.at[:, cols], wq_s.at[:, cols], sem_wq.at[g])

    def out_copy(t):
        cols = pl.ds(pl.multiple_of(t * 128, 128), 128)
        return pltpu.make_async_copy(x_s.at[:, cols], o_hbm.at[:, cols], sem_o.at[t])

    moda_copy = pltpu.make_async_copy(
        wmod_hbm.at[:, pl.ds(0, mod_a)], wmod_s.at[:, pl.ds(0, mod_a)], sem_w.at[0])
    modb_copy = pltpu.make_async_copy(
        wmod_hbm.at[:, pl.ds(mod_a, 4 * D)], wmod_s.at[:, pl.ds(mod_a, 4 * D)], sem_w.at[1])
    k_copy = pltpu.make_async_copy(k_hbm, k_s, sem_w.at[2])
    v_copy = pltpu.make_async_copy(v_hbm, v_s, sem_w.at[3])
    late_copies = [
        pltpu.make_async_copy(wg_hbm, wg_s, sem_w.at[4]),
        pltpu.make_async_copy(wu_hbm, wu_s, sem_w.at[5]),
        pltpu.make_async_copy(wd_hbm, wd_s, sem_w.at[6]),
    ] + [
        pltpu.make_async_copy(wo_hbm.at[:, pl.ds(h * DH, DH)], wo_s.at[h], sem_w.at[7 + h])
        for h in range(HQ)
    ]

    npan = -(-D // 128)
    qscale = (DH ** -0.5) * LOG2E

    def normalise(i, c):
        cols = pl.ds(pl.multiple_of(i * RB + c * 128, 128), 128)
        xv = x_s[:, cols].T.astype(F32)
        mean = jnp.sum(xv, axis=-1, keepdims=True) * (1.0 / D)
        xc = xv - mean
        var = jnp.sum(xc * xc, axis=-1, keepdims=True) * (1.0 / D)
        return xc * lax.rsqrt(var + LN_EPS)

    def put_h(slot, c, xn):
        hn = (xn * jnp.tile(ca1, (16, 1)) + jnp.tile(sa, (16, 1))).astype(BF16)
        for p in range(npan):
            w = min(128, D - p * 128)
            h_s[slot, p, c * 128:(c + 1) * 128, 0:w] = hn[:, p * 128:p * 128 + w]

    def ln1(i, slot):
        for c in range(RB // 128):
            put_h(slot, c, normalise(i, c))

    def get_h(slot):
        pans = [_unpack(h_i[slot, p]) for p in range(npan)]
        return jnp.concatenate(pans, axis=-1)[:, 0:D]

    def q_proj(i, slot, before=None):
        for j in range(nwq):
            if before is not None:
                before(j)
            q = jnp.dot(get_h(slot), wq_s[:, j * WQ_CHUNK:(j + 1) * WQ_CHUNK],
                        preferred_element_type=F32)
            for u in range(WQ_CHUNK // DH):
                q_s[j * (WQ_CHUNK // DH) + u, pl.ds(pl.multiple_of(i * RB, RB), RB), :] = (
                    q[:, u * DH:(u + 1) * DH] * qscale).astype(BF16)

    def fence():
        pl.semaphore_signal(sem_f, 1)
        pl.semaphore_wait(sem_f, 1)

    for cp in (x_copy(0), moda_copy, wq_copy(0), wq_copy(1), x_copy(1), wq_copy(2), wq_copy(3),
               x_copy(2), modb_copy, k_copy, v_copy):
        cp.start()
        fence()
    if D % 128:
        h_s[:, npan - 1] = jnp.zeros((2, RB, 128), BF16)
    cv = c_ref[...].astype(F32)
    sc = _rb(cv * _rb(jax.nn.sigmoid(cv)))
    sc = jnp.broadcast_to(sc, (16, D)).astype(BF16)

    x_copy(0).wait()
    for c in range(RB // 128):
        xn_s[c] = normalise(0, c)
    moda_copy.wait()
    mod = _rb(jnp.dot(sc, wmod_s[:, 0:mod_a], preferred_element_type=F32))[0:8]
    sa = mod[:, 0:D]
    ca1 = _rb(1.0 + mod[:, D:2 * D])
    for c in range(RB // 128):
        put_h(0, c, xn_s[c])

    def first_block(j):
        for g in range(len(WQ_GROUPS)):
            if j == g_lo[g]:
                wq_copy(g).wait()
                if g == 2:
                    x_copy(1).wait()
                    ln1(1, 1)

    q_proj(0, 0, first_block)
    x_copy(2).wait()

    def p1_body(i, carry):
        def mid(j):
            if j == nwq // 2:
                ln1(i + 1, (i + 1) & 1)

        q_proj(i, i & 1, mid)
        return carry

    lax.fori_loop(1, nrb - 1, p1_body, 0)

    modb_copy.wait()
    mod2 = _rb(jnp.dot(sc, wmod_s[:, mod_a:6 * D], preferred_element_type=F32))[0:8]
    gb = mod2[:, 3 * D:4 * D]
    for n, row in enumerate((mod2[:, 0:D], mod2[:, D:2 * D], _rb(1.0 + mod2[:, 2 * D:3 * D]), gb,
                             wr_ref[...].astype(F32))):
        col_s[n] = jnp.broadcast_to(row[0:1], (128, D)).T
    q_proj(nrb - 1, (nrb - 1) & 1)

    nbh = S // BQ
    nu = rep * nbh
    half = BQ // 2
    assert nu % 2 == 0

    def finish_max(slot):
        m = jnp.max(m_s[slot], axis=-1, keepdims=True)
        m_s[slot] = jnp.broadcast_to(m, (BQ, 128))

    def qk(h, u, defer):
        slot = u % 2
        q = _unpack(q_i[h * rep + u // nbh, (u % nbh) * half:(u % nbh + 1) * half, :])
        s = lax.dot_general(q, _unpack(k_i[h]), NT_DIMS, preferred_element_type=F32)
        s_s[slot] = s
        m_s[slot] = _fold(s, jnp.maximum)
        if not defer:
            finish_max(slot)

    def pv(h, u):
        slot = u % 2
        p = jnp.exp2(s_s[slot] - jnp.tile(m_s[slot], (1, S // 128)))
        l = jnp.sum(_fold(p, jnp.add), axis=-1, keepdims=True)
        acc = jnp.dot(p.astype(BF16), _unpack(v_i[h]), preferred_element_type=F32)
        inv = pl.reciprocal(l, approx=True)
        inv = inv * (2.0 - l * inv)
        o_s[h * rep + u // nbh, (u % nbh) * BQ:(u % nbh + 1) * BQ, :] = (acc * inv).astype(BF16)

    def p2_head(h, last):
        finish_max(1)
        for u in range(nu):
            pv(h, u)
            if u + 2 < nu:
                qk(h, u + 2, False)
            elif not last:
                qk(h + 1, u + 2 - nu, u == nu - 1)

    k_copy.wait()
    v_copy.wait()
    for cp in late_copies:
        cp.start()
    qk(0, 0, False)
    qk(0, 1, True)

    def p2_body(h, carry):
        p2_head(h, False)
        return carry

    lax.fori_loop(0, HKV - 1, p2_body, 0)
    p2_head(HKV - 1, True)

    ntb = S // TB
    for cp in late_copies:
        cp.wait()
    lanes = lambda a: jnp.tile(a, (1, TB // 128))

    def o_proj(i, kh):
        rows = pl.ds(pl.multiple_of(i * (TB // 2), TB // 2), TB // 2)
        h0, h1 = kh * HQ // 2, (kh + 1) * HQ // 2
        ob = jnp.concatenate([_unpack(o_i[h, rows, :]) for h in range(h0, h1)], axis=-1)
        wt = jnp.concatenate([_unpack(wo_i[h]) for h in range(h0, h1)], axis=-1)
        return lax.dot_general(wt, ob, NT_DIMS, preferred_element_type=F32)

    def resid_norm(i, a):
        cols = pl.ds(pl.multiple_of(i * TB, TB), TB)
        x1 = _rb(x_s[:, cols].astype(F32) + lanes(col_s[0]) * a)
        mean = jnp.sum(x1, axis=0, keepdims=True) * (1.0 / D)
        xc = x1 - mean
        var = jnp.sum(xc * xc, axis=0, keepdims=True) * (1.0 / D)
        std = _rb(jnp.sqrt(_rb(_rb(var) + LN_EPS_BF16)))
        hn = _rb(_rb(x1 - _rb(mean)) / std)
        h2 = _rb(_rb(hn * lanes(col_s[2])) + lanes(col_s[1]))
        h2r_s[cols, :] = h2.astype(BF16).T
        x_s[:, cols] = (x1 + lanes(col_s[3]) * h2).astype(BF16)
        r = jnp.sum(h2 * lanes(col_s[4]), axis=0, keepdims=True)
        r_s[:, cols] = jnp.broadcast_to(_rb(r), (8, TB))
        for u in range(TB // 128):
            out_copy(i * (TB // 128) + u).start()

    a_s[...] = o_proj(0, 0) + o_proj(0, 1)

    def p3_body(i, carry):
        a = a_s[...]
        a_s[...] = o_proj(i + 1, 0)
        resid_norm(i, a)
        a_s[...] += o_proj(i + 1, 1)
        return carry

    lax.fori_loop(0, ntb - 1, p3_body, 0)
    resid_norm(ntb - 1, a_s[...])

    r = r_s[...]
    col = lax.broadcasted_iota(I32, (8, S), 1)
    rbits = pltpu.bitcast(r, I32)
    key = pltpu.bitcast(rbits | jnp.where(rbits >= 0, (S - 1) - col, col), F32)
    sub = lax.broadcasted_iota(I32, (8, 128), 0)
    keyc = []
    for g in range(S // 1024):
        kc = key[:, g * 1024:g * 1024 + 128]
        for u in range(1, 8):
            kc = jnp.where(sub == u, key[:, g * 1024 + u * 128:g * 1024 + (u + 1) * 128], kc)
        keyc.append(kc)

    def token_row(ref, idx):
        word = ref[pl.ds(idx // 2, 1), :]
        bits = jnp.where(idx % 2 == 0, word << 16, word & jnp.int32(-65536))
        return pltpu.bitcast(jnp.broadcast_to(bits, (8, D)), F32)

    sub_d = lax.broadcasted_iota(I32, (8, D), 0)
    xsel = jnp.zeros((8, D), F32)
    best = jnp.zeros((8, 128), F32)
    idxs = []
    for j in range(TOPC):
        mx = functools.reduce(jnp.maximum, keyc)
        mx = jnp.max(jnp.max(mx, axis=0, keepdims=True), axis=1, keepdims=True)
        mxb = jnp.broadcast_to(mx, (8, 128))
        keyc = [jnp.where(kc == mxb, -jnp.inf, kc) for kc in keyc]
        best = jnp.where(sub == j, mxb, best)
        mb = pltpu.bitcast(mxb, I32)
        low = mb & (S - 1)
        idx = jnp.max(jnp.where(mb >= 0, (S - 1) - low, low))
        idxs.append(idx)
        xsel = jnp.where(sub_d == j, token_row(h2r_s.bitcast(I32), idx), xsel)

    rsel = pltpu.bitcast(pltpu.bitcast(best, I32) & jnp.int32(-65536), F32)[:, 0:1]
    xs = jnp.concatenate([xsel, xsel], axis=0).astype(BF16)
    g = _rb(jnp.dot(xs, wg_s[...], preferred_element_type=F32)[0:8])
    up = _rb(jnp.dot(xs, wu_s[...], preferred_element_type=F32)[0:8])
    act = _rb(_rb(g * _rb(jax.nn.sigmoid(g))) * up)
    act = jnp.concatenate([act, act], axis=0).astype(BF16)
    y = _rb(lax.dot_general(act, wd_s[...], NT_DIMS, preferred_element_type=F32)[0:8])
    y = _rb(y * _rb(jax.nn.sigmoid(rsel)))
    upd = gb * (_rb(xsel + y) - xsel)

    updc = jnp.concatenate([upd, jnp.zeros((120, D), F32)], axis=0).T
    for t in range(S // 128):
        out_copy(t).wait()
    lane = lax.broadcasted_iota(I32, updc.shape, 1)
    for j in range(TOPC):
        cols = pl.ds(pl.multiple_of((idxs[j] // 128) * 128, 128), 128)
        moved = pltpu.roll(updc, (idxs[j] - j) % 128, 1)
        old = x_s[:, cols].astype(F32)
        x_s[:, cols] = jnp.where(lane == idxs[j] % 128, old + moved, old).astype(BF16)

    tiles = [idx // 128 for idx in idxs]
    hits = [functools.reduce(jnp.logical_or, [tl == t for tl in tiles]) for t in range(S // 128)]
    for t in range(S // 128):
        @pl.when(hits[t])
        def _():
            out_copy(t).start()
    for t in range(S // 128):
        @pl.when(hits[t])
        def _():
            out_copy(t).wait()


@jax.jit
def pallas_adaLN_cond__gqa_block_cached__moe_arch_mod__prompt_kernel(
    A_x: jax.Array,
    A_k_cache: jax.Array,
    A_v_cache: jax.Array,
    A_wq: jax.Array,
    A_wo: jax.Array,
    B_x: jax.Array,
    B_w_r: jax.Array,
    B_w_gate: jax.Array,
    B_w_up: jax.Array,
    B_w_down: jax.Array,
    c: jax.Array,
    w_mod: jax.Array,
):
    del B_x
    B, S, D = A_x.shape
    _, HKV, SK, DH = A_k_cache.shape
    HQ = A_wq.shape[1] // DH
    F = B_w_gate.shape[1]
    assert B == 1 and SK == S and DH == 128 and S % 1024 == 0 and S <= 65536

    vm = pltpu.VMEM
    dma = pltpu.SemaphoreType.DMA
    hbm = pl.BlockSpec(memory_space=pl.ANY)
    small = pl.BlockSpec(memory_space=pltpu.VMEM)
    out = pl.pallas_call(
        functools.partial(_kernel, S=S, D=D, HQ=HQ, HKV=HKV, DH=DH),
        out_shape=jax.ShapeDtypeStruct((D, S), BF16),
        in_specs=[small, small] + [hbm] * 9,
        out_specs=hbm,
        scratch_shapes=[
            vm((D, S), BF16),
            vm((HKV, S, DH), BF16),
            vm((HKV, S, DH), BF16),
            vm((D, HQ * DH), BF16),
            vm((HQ, D, DH), BF16),
            vm((D, F), BF16),
            vm((D, F), BF16),
            vm((D, F), BF16),
            vm((D, 6 * D), BF16),
            vm((HQ, S, DH), BF16),
            vm((HQ, S, DH), BF16),
            vm((2, BQ, S), F32),
            vm((2, BQ, 128), F32),
            vm((2, -(-D // 128), RB, 128), BF16),
            vm((RB // 128, 128, D), F32),
            vm((D, TB), F32),
            vm((5, D, 128), F32),
            vm((S, D), BF16),
            vm((8, S), F32),
            dma((3,)), dma((len(WQ_GROUPS),)), dma((7 + HQ,)), dma((S // 128,)),
            pltpu.SemaphoreType.REGULAR,
        ],
        compiler_params=pltpu.CompilerParams(
            vmem_limit_bytes=118 * 1024 * 1024,
            flags={"XLA_TPU_FORCE_LP_LLO_SCHEDULER": True},
        ),
        name="adaln_gqa_moe_block",
    )(c, B_w_r.reshape(1, D), A_x[0].T, A_k_cache[0], A_v_cache[0], A_wq, A_wo.T,
      B_w_gate, B_w_up, B_w_down.T, w_mod)
    return out.T[None]
```

```python
import functools

import jax
import jax.numpy as jnp
import jax.experimental.pallas as pl
import jax.experimental.pallas.tpu as pltpu
import numpy as np
from jax import lax

F32 = jnp.float32
BF16 = jnp.bfloat16
I32 = jnp.int32

NT_DIMS = (((1,), (1,)), ((), ()))
TOPC = 8
LN_EPS = 1e-5
LN_EPS_BF16 = float(np.asarray(LN_EPS, dtype=jnp.bfloat16))
LOG2E = 1.4426950408889634

RB = 512
BQ = 512
TB = 256
WQ_CHUNK = 512
WQ_GROUPS = (1, 2, 4, 1)


def _rb(a):
    return a.astype(BF16).astype(F32)


def _unpack(a):
    return pltpu.bitcast(a, BF16)


def _fold(a, op):
    out = a[:, :128]
    for j in range(1, a.shape[1] // 128):
        out = op(out, a[:, j * 128:(j + 1) * 128])
    return out


def _kernel(c_hbm, wr_hbm, x_hbm, k_hbm, v_hbm, wq_hbm, wo_hbm, wg_hbm, wu_hbm, wd_hbm,
            wmod_hbm, o_hbm,
            x_s, k_s, v_s, wq_s, wo_s, wg_s, wu_s, wd_s, wmod_s,
            q_s, o_s, s_s, m_s, h_s, xn_s, ms_s, a_s, col_s, h2r_s, r_s, c_s, wr_s,
            sem_x, sem_wq, sem_w, sem_o, sem_c, sem_f,
            *, S, D, HQ, HKV, DH):
    mod_a = 2 * D
    rep = HQ // HKV
    k_i = k_s.bitcast(I32)
    v_i = v_s.bitcast(I32)
    q_i = q_s.bitcast(I32)
    o_i = o_s.bitcast(I32)
    h_i = h_s.bitcast(I32)
    wo_i = wo_s.bitcast(I32)

    nrb = S // RB
    nwq = HQ * DH // WQ_CHUNK
    assert sum(WQ_GROUPS) == nwq and nrb >= 3
    g_lo = np.cumsum((0,) + WQ_GROUPS)

    def x_copy(g):
        cols = pl.ds(g * RB, RB if g < 2 else S - 2 * RB)
        return pltpu.make_async_copy(x_hbm.at[:, cols], x_s.at[:, cols], sem_x.at[g])

    def wq_copy(g):
        cols = pl.ds(int(g_lo[g]) * WQ_CHUNK, WQ_GROUPS[g] * WQ_CHUNK)
        return pltpu.make_async_copy(wq_hbm.at[:, cols], wq_s.at[:, cols], sem_wq.at[g])

    def out_copy(t):
        cols = pl.ds(pl.multiple_of(t * 128, 128), 128)
        return pltpu.make_async_copy(x_s.at[:, cols], o_hbm.at[:, cols], sem_o.at[t])

    moda_copy = pltpu.make_async_copy(
        wmod_hbm.at[:, pl.ds(0, mod_a)], wmod_s.at[:, pl.ds(0, mod_a)], sem_w.at[0])
    modb_copy = pltpu.make_async_copy(
        wmod_hbm.at[:, pl.ds(mod_a, 4 * D)], wmod_s.at[:, pl.ds(mod_a, 4 * D)], sem_w.at[1])
    c_copy = pltpu.make_async_copy(c_hbm, c_s, sem_c.at[0])
    wr_copy = pltpu.make_async_copy(wr_hbm, wr_s, sem_c.at[1])
    k_copy = pltpu.make_async_copy(k_hbm, k_s, sem_w.at[2])
    v_copy = pltpu.make_async_copy(v_hbm, v_s, sem_w.at[3])
    late_copies = [
        pltpu.make_async_copy(wg_hbm, wg_s, sem_w.at[4]),
        pltpu.make_async_copy(wu_hbm, wu_s, sem_w.at[5]),
        pltpu.make_async_copy(wd_hbm, wd_s, sem_w.at[6]),
    ] + [
        pltpu.make_async_copy(wo_hbm.at[:, pl.ds(h * DH, DH)], wo_s.at[h], sem_w.at[7 + h])
        for h in range(HQ)
    ]

    npan = -(-D // 128)
    qscale = (DH ** -0.5) * LOG2E

    def normalise(i, c):
        cols = pl.ds(pl.multiple_of(i * RB + c * 128, 128), 128)
        xv = x_s[:, cols].T.astype(F32)
        mean = jnp.sum(xv, axis=-1, keepdims=True) * (1.0 / D)
        xc = xv - mean
        var = jnp.sum(xc * xc, axis=-1, keepdims=True) * (1.0 / D)
        return xc * lax.rsqrt(var + LN_EPS)

    def put_h(slot, c, xn):
        hn = xn * jnp.tile(ms_s[0], (16, 1)) + jnp.tile(ms_s[1], (16, 1))
        if D % 128:
            hn = jnp.concatenate([hn, jnp.zeros((128, npan * 128 - D), F32)], axis=-1)
        for p in range(npan):
            h_s[slot, p, c * 128:(c + 1) * 128, :] = hn[:, p * 128:(p + 1) * 128].astype(BF16)

    def ln1(i, slot):
        for c in range(RB // 128):
            put_h(slot, c, normalise(i, c))

    def get_h(slot):
        pans = [_unpack(h_i[slot, p]) for p in range(npan)]
        return jnp.concatenate(pans, axis=-1)[:, 0:D]

    def q_proj(i, slot, before=None):
        for j in range(nwq):
            if before is not None:
                before(j)
            q = jnp.dot(get_h(slot), wq_s[:, j * WQ_CHUNK:(j + 1) * WQ_CHUNK],
                        preferred_element_type=F32)
            for u in range(WQ_CHUNK // DH):
                q_s[j * (WQ_CHUNK // DH) + u, pl.ds(pl.multiple_of(i * RB, RB), RB), :] = (
                    q[:, u * DH:(u + 1) * DH] * qscale).astype(BF16)

    def fence():
        pl.semaphore_signal(sem_f, 1)
        pl.semaphore_wait(sem_f, 1)

    for cp in (c_copy, x_copy(0), moda_copy, wq_copy(0), wq_copy(1), x_copy(1), wq_copy(2), wq_copy(3),
               x_copy(2), wr_copy, modb_copy, k_copy, v_copy):
        cp.start()
        fence()
    c_copy.wait()
    x_copy(0).wait()
    cv = c_s[...].astype(F32)
    sc = _rb(cv * _rb(jax.nn.sigmoid(cv)))
    sc = jnp.broadcast_to(sc, (16, D)).astype(BF16)
    for c in range(RB // 128):
        xn_s[c] = normalise(0, c)
    moda_copy.wait()
    mod = _rb(jnp.dot(sc, wmod_s[:, 0:mod_a], preferred_element_type=F32))[0:8]
    ms_s[0] = _rb(1.0 + mod[:, D:2 * D])
    ms_s[1] = mod[:, 0:D]
    fence()
    for c in range(RB // 128):
        put_h(0, c, xn_s[c])
        fence()

    def first_block(j):
        for g in range(len(WQ_GROUPS)):
            if j == g_lo[g]:
                wq_copy(g).wait()
                if g == 2:
                    x_copy(1).wait()
                    ln1(1, 1)

    q_proj(0, 0, first_block)
    x_copy(2).wait()

    def p1_body(i, carry):
        def mid(j):
            if j == nwq // 2:
                ln1(i + 1, (i + 1) & 1)

        q_proj(i, i & 1, mid)
        return carry

    lax.fori_loop(1, nrb - 1, p1_body, 0)

    wr_copy.wait()
    modb_copy.wait()
    k_copy.wait()
    v_copy.wait()
    for cp in late_copies:
        cp.start()
    mod2 = _rb(jnp.dot(sc, wmod_s[:, mod_a:6 * D], preferred_element_type=F32))[0:8]
    gb = mod2[:, 3 * D:4 * D]
    for n, row in enumerate((mod2[:, 0:D], mod2[:, D:2 * D], _rb(1.0 + mod2[:, 2 * D:3 * D]), gb,
                             wr_s[...].astype(F32).reshape(1, D))):
        col_s[n] = jnp.broadcast_to(row[0:1], (128, D)).T
    q_proj(nrb - 1, (nrb - 1) & 1)

    nbh = S // BQ
    nu = rep * nbh
    half = BQ // 2
    assert nu % 2 == 0

    def finish_max(slot):
        m = jnp.max(m_s[slot], axis=-1, keepdims=True)
        m_s[slot] = jnp.broadcast_to(m, (BQ, 128))

    def qk(h, u, defer):
        slot = u % 2
        q = _unpack(q_i[h * rep + u // nbh, (u % nbh) * half:(u % nbh + 1) * half, :])
        s = lax.dot_general(q, _unpack(k_i[h]), NT_DIMS, preferred_element_type=F32)
        s_s[slot] = s
        m_s[slot] = _fold(s, jnp.maximum)
        if not defer:
            finish_max(slot)

    def pv(h, u):
        slot = u % 2
        p = jnp.exp2(s_s[slot] - jnp.tile(m_s[slot], (1, S // 128)))
        l = jnp.sum(_fold(p, jnp.add), axis=-1, keepdims=True)
        acc = jnp.dot(p.astype(BF16), _unpack(v_i[h]), preferred_element_type=F32)
        inv = pl.reciprocal(l, approx=True)
        inv = inv * (2.0 - l * inv)
        o_s[h * rep + u // nbh, (u % nbh) * BQ:(u % nbh + 1) * BQ, :] = (acc * inv).astype(BF16)

    def p2_head(h, last):
        finish_max(1)
        for u in range(nu):
            pv(h, u)
            if u + 2 < nu:
                qk(h, u + 2, False)
            elif not last:
                qk(h + 1, u + 2 - nu, u == nu - 1)

    qk(0, 0, False)
    qk(0, 1, True)

    def p2_body(h, carry):
        p2_head(h, False)
        return carry

    lax.fori_loop(0, HKV - 1, p2_body, 0)
    for cp in late_copies:
        cp.wait()
    p2_head(HKV - 1, True)

    ntb = S // TB
    lanes = lambda a: jnp.tile(a, (1, TB // 128))

    def o_proj(i, kh):
        rows = pl.ds(pl.multiple_of(i * (TB // 2), TB // 2), TB // 2)
        h0, h1 = kh * HQ // 2, (kh + 1) * HQ // 2
        ob = jnp.concatenate([_unpack(o_i[h, rows, :]) for h in range(h0, h1)], axis=-1)
        wt = jnp.concatenate([_unpack(wo_i[h]) for h in range(h0, h1)], axis=-1)
        return lax.dot_general(wt, ob, NT_DIMS, preferred_element_type=F32)

    def resid_norm(i, a):
        cols = pl.ds(pl.multiple_of(i * TB, TB), TB)
        x1 = _rb(x_s[:, cols].astype(F32) + lanes(col_s[0]) * a)
        mean = jnp.sum(x1, axis=0, keepdims=True) * (1.0 / D)
        xc = x1 - mean
        var = jnp.sum(xc * xc, axis=0, keepdims=True) * (1.0 / D)
        std = _rb(jnp.sqrt(_rb(_rb(var) + LN_EPS_BF16)))
        hn = _rb(_rb(x1 - _rb(mean)) / std)
        h2 = _rb(_rb(hn * lanes(col_s[2])) + lanes(col_s[1]))
        h2r_s[cols, :] = h2.astype(BF16).T
        x_s[:, cols] = (x1 + lanes(col_s[3]) * h2).astype(BF16)
        r = jnp.sum(h2 * lanes(col_s[4]), axis=0, keepdims=True)
        r_s[:, cols] = jnp.broadcast_to(_rb(r), (8, TB))
        for u in range(TB // 128):
            out_copy(i * (TB // 128) + u).start()

    a_s[...] = o_proj(0, 0) + o_proj(0, 1)

    def p3_body(i, carry):
        a = a_s[...]
        a_s[...] = o_proj(i + 1, 0)
        resid_norm(i, a)
        a_s[...] += o_proj(i + 1, 1)
        return carry

    lax.fori_loop(0, ntb - 1, p3_body, 0)
    resid_norm(ntb - 1, a_s[...])

    r = r_s[...]
    col = lax.broadcasted_iota(I32, (8, S), 1)
    rbits = pltpu.bitcast(r, I32)
    key = pltpu.bitcast(rbits | jnp.where(rbits >= 0, (S - 1) - col, col), F32)
    sub = lax.broadcasted_iota(I32, (8, 128), 0)
    keyc = []
    for g in range(S // 1024):
        kc = key[:, g * 1024:g * 1024 + 128]
        for u in range(1, 8):
            kc = jnp.where(sub == u, key[:, g * 1024 + u * 128:g * 1024 + (u + 1) * 128], kc)
        keyc.append(kc)

    def token_row(ref, idx):
        word = ref[pl.ds(idx // 2, 1), :]
        bits = jnp.where(idx % 2 == 0, word << 16, word & jnp.int32(-65536))
        return pltpu.bitcast(jnp.broadcast_to(bits, (8, D)), F32)

    sub_d = lax.broadcasted_iota(I32, (8, D), 0)
    xsel = jnp.zeros((8, D), F32)
    best = jnp.zeros((8, 128), F32)
    idxs = []
    for j in range(TOPC):
        mx = functools.reduce(jnp.maximum, keyc)
        mx = jnp.max(jnp.max(mx, axis=0, keepdims=True), axis=1, keepdims=True)
        mxb = jnp.broadcast_to(mx, (8, 128))
        keyc = [jnp.where(kc == mxb, -jnp.inf, kc) for kc in keyc]
        best = jnp.where(sub == j, mxb, best)
        mb = pltpu.bitcast(mxb, I32)
        low = mb & (S - 1)
        idx = jnp.max(jnp.where(mb >= 0, (S - 1) - low, low))
        idxs.append(idx)
        xsel = jnp.where(sub_d == j, token_row(h2r_s.bitcast(I32), idx), xsel)

    rsel = pltpu.bitcast(pltpu.bitcast(best, I32) & jnp.int32(-65536), F32)[:, 0:1]
    xs = jnp.concatenate([xsel, xsel], axis=0).astype(BF16)
    g = _rb(jnp.dot(xs, wg_s[...], preferred_element_type=F32)[0:8])
    up = _rb(jnp.dot(xs, wu_s[...], preferred_element_type=F32)[0:8])
    act = _rb(_rb(g * _rb(jax.nn.sigmoid(g))) * up)
    act = jnp.concatenate([act, act], axis=0).astype(BF16)
    y = _rb(lax.dot_general(act, wd_s[...], NT_DIMS, preferred_element_type=F32)[0:8])
    y = _rb(y * _rb(jax.nn.sigmoid(rsel)))
    upd = gb * (_rb(xsel + y) - xsel)

    updc = jnp.concatenate([upd, jnp.zeros((120, D), F32)], axis=0).T
    for t in range(S // 128):
        out_copy(t).wait()
    lane = lax.broadcasted_iota(I32, updc.shape, 1)
    for j in range(TOPC):
        cols = pl.ds(pl.multiple_of((idxs[j] // 128) * 128, 128), 128)
        moved = pltpu.roll(updc, (idxs[j] - j) % 128, 1)
        old = x_s[:, cols].astype(F32)
        x_s[:, cols] = jnp.where(lane == idxs[j] % 128, old + moved, old).astype(BF16)

    tiles = [idx // 128 for idx in idxs]
    hits = [functools.reduce(jnp.logical_or, [tl == t for tl in tiles]) for t in range(S // 128)]
    for t in range(S // 128):
        @pl.when(hits[t])
        def _():
            out_copy(t).start()
    for t in range(S // 128):
        @pl.when(hits[t])
        def _():
            out_copy(t).wait()


@jax.jit
def pallas_adaLN_cond__gqa_block_cached__moe_arch_mod__prompt_kernel(
    A_x: jax.Array,
    A_k_cache: jax.Array,
    A_v_cache: jax.Array,
    A_wq: jax.Array,
    A_wo: jax.Array,
    B_x: jax.Array,
    B_w_r: jax.Array,
    B_w_gate: jax.Array,
    B_w_up: jax.Array,
    B_w_down: jax.Array,
    c: jax.Array,
    w_mod: jax.Array,
):
    del B_x
    B, S, D = A_x.shape
    _, HKV, SK, DH = A_k_cache.shape
    HQ = A_wq.shape[1] // DH
    F = B_w_gate.shape[1]
    assert B == 1 and SK == S and DH == 128 and S % 1024 == 0 and S <= 65536

    vm = pltpu.VMEM
    dma = pltpu.SemaphoreType.DMA
    hbm = pl.BlockSpec(memory_space=pl.ANY)
    out = pl.pallas_call(
        functools.partial(_kernel, S=S, D=D, HQ=HQ, HKV=HKV, DH=DH),
        out_shape=jax.ShapeDtypeStruct((D, S), BF16),
        in_specs=[hbm] * 11,
        out_specs=hbm,
        scratch_shapes=[
            vm((D, S), BF16),
            vm((HKV, S, DH), BF16),
            vm((HKV, S, DH), BF16),
            vm((D, HQ * DH), BF16),
            vm((HQ, D, DH), BF16),
            vm((D, F), BF16),
            vm((D, F), BF16),
            vm((D, F), BF16),
            vm((D, 6 * D), BF16),
            vm((HQ, S, DH), BF16),
            vm((HQ, S, DH), BF16),
            vm((2, BQ, S), F32),
            vm((2, BQ, 128), F32),
            vm((2, -(-D // 128), RB, 128), BF16),
            vm((RB // 128, 128, D), F32),
            vm((2, 8, D), F32),
            vm((D, TB), F32),
            vm((5, D, 128), F32),
            vm((S, D), BF16),
            vm((8, S), F32),
            vm((1, D), BF16),
            vm((D,), BF16),
            dma((3,)), dma((len(WQ_GROUPS),)), dma((7 + HQ,)), dma((S // 128,)), dma((2,)),
            pltpu.SemaphoreType.REGULAR,
        ],
        compiler_params=pltpu.CompilerParams(
            vmem_limit_bytes=118 * 1024 * 1024,
            flags={"XLA_TPU_FORCE_LP_LLO_SCHEDULER": True},
        ),
        name="adaln_gqa_moe_block",
    )(c, B_w_r, A_x[0].T, A_k_cache[0], A_v_cache[0], A_wq, A_wo.T,
      B_w_gate, B_w_up, B_w_down.T, w_mod)
    return out.T[None]
```

```python
import functools

import jax
import jax.numpy as jnp
import jax.experimental.pallas as pl
import jax.experimental.pallas.tpu as pltpu
import numpy as np
from jax import lax

F32 = jnp.float32
BF16 = jnp.bfloat16
I32 = jnp.int32

NT_DIMS = (((1,), (1,)), ((), ()))
TOPC = 8
LN_EPS = 1e-5
LN_EPS_BF16 = float(np.asarray(LN_EPS, dtype=jnp.bfloat16))
LOG2E = 1.4426950408889634

RB = 512
BQ = 256
TB = 256
WQ_CHUNK = 512
WQ_GROUPS = (1, 2, 4, 1)


def _rb(a):
    return a.astype(BF16).astype(F32)


def _unpack(a):
    return pltpu.bitcast(a, BF16)


def _fold(a, op):
    out = a[:, :128]
    for j in range(1, a.shape[1] // 128):
        out = op(out, a[:, j * 128:(j + 1) * 128])
    return out


def _kernel(c_hbm, wr_hbm, x_hbm, k_hbm, v_hbm, wq_hbm, wo_hbm, wg_hbm, wu_hbm, wd_hbm,
            wmod_hbm, o_hbm,
            x_s, k_s, v_s, wq_s, wo_s, wg_s, wu_s, wd_s, wmod_s,
            q_s, o_s, s_s, m_s, h_s, xn_s, ms_s, a_s, col_s, h2r_s, key_s, wdt_s, patch_s,
            c_s, wr_s,
            sem_x, sem_wq, sem_w, sem_o, sem_c, sem_p, sem_f,
            *, S, D, HQ, HKV, DH, F):
    mod_a = 2 * D
    rep = HQ // HKV
    k_i = k_s.bitcast(I32)
    v_i = v_s.bitcast(I32)
    q_i = q_s.bitcast(I32)
    o_i = o_s.bitcast(I32)
    h_i = h_s.bitcast(I32)
    wo_i = wo_s.bitcast(I32)

    nrb = S // RB
    nwq = HQ * DH // WQ_CHUNK
    assert sum(WQ_GROUPS) == nwq and nrb >= 3
    g_lo = np.cumsum((0,) + WQ_GROUPS)

    def x_copy(g):
        cols = pl.ds(g * RB, RB if g < 2 else S - 2 * RB)
        return pltpu.make_async_copy(x_hbm.at[:, cols], x_s.at[:, cols], sem_x.at[g])

    def wq_copy(g):
        cols = pl.ds(int(g_lo[g]) * WQ_CHUNK, WQ_GROUPS[g] * WQ_CHUNK)
        return pltpu.make_async_copy(wq_hbm.at[:, cols], wq_s.at[:, cols], sem_wq.at[g])

    def out_copy(t):
        cols = pl.ds(pl.multiple_of(t * 128, 128), 128)
        return pltpu.make_async_copy(x_s.at[:, cols], o_hbm.at[:, cols], sem_o.at[t])

    moda_copy = pltpu.make_async_copy(
        wmod_hbm.at[:, pl.ds(0, mod_a)], wmod_s.at[:, pl.ds(0, mod_a)], sem_w.at[0])
    modb_copy = pltpu.make_async_copy(
        wmod_hbm.at[:, pl.ds(mod_a, 4 * D)], wmod_s.at[:, pl.ds(mod_a, 4 * D)], sem_w.at[1])
    c_copy = pltpu.make_async_copy(c_hbm, c_s, sem_c.at[0])
    wr_copy = pltpu.make_async_copy(wr_hbm, wr_s, sem_c.at[1])
    k_copy = pltpu.make_async_copy(k_hbm, k_s, sem_w.at[2])
    v_copy = pltpu.make_async_copy(v_hbm, v_s, sem_w.at[3])
    late_copies = [
        pltpu.make_async_copy(wg_hbm, wg_s, sem_w.at[4]),
        pltpu.make_async_copy(wu_hbm, wu_s, sem_w.at[5]),
        pltpu.make_async_copy(wd_hbm, wd_s, sem_w.at[6]),
    ] + [
        pltpu.make_async_copy(wo_hbm.at[:, pl.ds(h * DH, DH)], wo_s.at[h], sem_w.at[7 + h])
        for h in range(HQ)
    ]

    npan = -(-D // 128)
    qscale = (DH ** -0.5) * LOG2E

    def normalise(i, c):
        cols = pl.ds(pl.multiple_of(i * RB + c * 128, 128), 128)
        xv = x_s[:, cols].T.astype(F32)
        mean = jnp.sum(xv, axis=-1, keepdims=True) * (1.0 / D)
        xc = xv - mean
        var = jnp.sum(xc * xc, axis=-1, keepdims=True) * (1.0 / D)
        return xc * lax.rsqrt(var + LN_EPS)

    def put_h(slot, c, xn):
        hn = xn * jnp.tile(ms_s[0], (16, 1)) + jnp.tile(ms_s[1], (16, 1))
        if D % 128:
            hn = jnp.concatenate([hn, jnp.zeros((128, npan * 128 - D), F32)], axis=-1)
        for p in range(npan):
            h_s[slot, p, c * 128:(c + 1) * 128, :] = hn[:, p * 128:(p + 1) * 128].astype(BF16)

    def ln1(i, slot):
        for c in range(RB // 128):
            put_h(slot, c, normalise(i, c))

    def get_h(slot):
        pans = [_unpack(h_i[slot, p]) for p in range(npan)]
        return jnp.concatenate(pans, axis=-1)[:, 0:D]

    def q_proj(i, slot, before=None):
        for j in range(nwq):
            if before is not None:
                before(j)
            q = jnp.dot(get_h(slot), wq_s[:, j * WQ_CHUNK:(j + 1) * WQ_CHUNK],
                        preferred_element_type=F32)
            for u in range(WQ_CHUNK // DH):
                q_s[j * (WQ_CHUNK // DH) + u, pl.ds(pl.multiple_of(i * RB, RB), RB), :] = (
                    q[:, u * DH:(u + 1) * DH] * qscale).astype(BF16)

    def fence():
        pl.semaphore_signal(sem_f, 1)
        pl.semaphore_wait(sem_f, 1)

    for cp in (c_copy, x_copy(0), moda_copy, wq_copy(0), wq_copy(1), x_copy(1), wq_copy(2), wq_copy(3),
               x_copy(2), wr_copy, modb_copy, k_copy, v_copy):
        cp.start()
        fence()
    c_copy.wait()
    x_copy(0).wait()
    cv = c_s[...].astype(F32)
    sc = _rb(cv * _rb(jax.nn.sigmoid(cv)))
    sc = jnp.broadcast_to(sc, (16, D)).astype(BF16)
    for c in range(RB // 128):
        xn_s[c] = normalise(0, c)
    moda_copy.wait()
    mod = _rb(jnp.dot(sc, wmod_s[:, 0:mod_a], preferred_element_type=F32))[0:8]
    ms_s[0] = _rb(1.0 + mod[:, D:2 * D])
    ms_s[1] = mod[:, 0:D]
    fence()
    for c in range(RB // 128):
        put_h(0, c, xn_s[c])
        fence()

    def first_block(j):
        for g in range(len(WQ_GROUPS)):
            if j == g_lo[g]:
                wq_copy(g).wait()
                if g == 2:
                    x_copy(1).wait()
                    ln1(1, 1)

    q_proj(0, 0, first_block)
    x_copy(2).wait()

    def p1_body(i, carry):
        def mid(j):
            if j == nwq // 2:
                ln1(i + 1, (i + 1) & 1)

        q_proj(i, i & 1, mid)
        return carry

    lax.fori_loop(1, nrb - 1, p1_body, 0)

    wr_copy.wait()
    modb_copy.wait()
    k_copy.wait()
    v_copy.wait()
    for cp in late_copies:
        cp.start()
    mod2 = _rb(jnp.dot(sc, wmod_s[:, mod_a:6 * D], preferred_element_type=F32))[0:8]
    gb = mod2[:, 3 * D:4 * D]
    for n, row in enumerate((mod2[:, 0:D], mod2[:, D:2 * D], _rb(1.0 + mod2[:, 2 * D:3 * D]), gb,
                             wr_s[...].astype(F32).reshape(1, D))):
        col_s[n] = jnp.broadcast_to(row[0:1], (128, D)).T
    q_proj(nrb - 1, (nrb - 1) & 1)

    nbh = S // BQ
    nu = rep * nbh
    half = BQ // 2
    assert nu % 2 == 0

    def finish_max(slot):
        m = jnp.max(m_s[slot], axis=-1, keepdims=True)
        m_s[slot] = jnp.broadcast_to(m, (BQ, 128))

    def qk(h, u, defer):
        slot = u % 2
        q = _unpack(q_i[h * rep + u // nbh, (u % nbh) * half:(u % nbh + 1) * half, :])
        s = lax.dot_general(q, _unpack(k_i[h]), NT_DIMS, preferred_element_type=F32)
        s_s[slot] = s
        m_s[slot] = _fold(s, jnp.maximum)
        if not defer:
            finish_max(slot)

    def pv(h, u):
        slot = u % 2
        p = jnp.exp2(s_s[slot] - jnp.tile(m_s[slot], (1, S // 128)))
        l = jnp.sum(_fold(p, jnp.add), axis=-1, keepdims=True)
        acc = jnp.dot(p.astype(BF16), _unpack(v_i[h]), preferred_element_type=F32)
        inv = pl.reciprocal(l, approx=True)
        inv = inv * (2.0 - l * inv)
        o_s[h * rep + u // nbh, (u % nbh) * BQ:(u % nbh + 1) * BQ, :] = (acc * inv).astype(BF16)

    def p2_head(h, last):
        finish_max(1)
        for u in range(nu):
            pv(h, u)
            if u + 2 < nu:
                qk(h, u + 2, False)
            elif not last:
                qk(h + 1, u + 2 - nu, u == nu - 1)

    qk(0, 0, False)
    qk(0, 1, True)

    def p2_body(h, carry):
        p2_head(h, False)
        return carry

    lax.fori_loop(0, HKV - 1, p2_body, 0)
    for cp in late_copies:
        cp.wait()
    for j in range(F // 128):
        wdt_s[j * 128:(j + 1) * 128, :] = wd_s[:, j * 128:(j + 1) * 128].T
    p2_head(HKV - 1, True)

    ntb = S // TB
    lanes = lambda a: jnp.tile(a, (1, TB // 128))

    def o_proj(i, kh):
        rows = pl.ds(pl.multiple_of(i * (TB // 2), TB // 2), TB // 2)
        h0, h1 = kh * HQ // 2, (kh + 1) * HQ // 2
        ob = jnp.concatenate([_unpack(o_i[h, rows, :]) for h in range(h0, h1)], axis=-1)
        wt = jnp.concatenate([_unpack(wo_i[h]) for h in range(h0, h1)], axis=-1)
        return lax.dot_general(wt, ob, NT_DIMS, preferred_element_type=F32)

    def resid_norm(i, a):
        cols = pl.ds(pl.multiple_of(i * TB, TB), TB)
        x1 = _rb(x_s[:, cols].astype(F32) + lanes(col_s[0]) * a)
        mean = jnp.sum(x1, axis=0, keepdims=True) * (1.0 / D)
        xc = x1 - mean
        var = jnp.sum(xc * xc, axis=0, keepdims=True) * (1.0 / D)
        std = _rb(jnp.sqrt(_rb(_rb(var) + LN_EPS_BF16)))
        hn = _rb(_rb(x1 - _rb(mean)) / std)
        h2 = _rb(_rb(hn * lanes(col_s[2])) + lanes(col_s[1]))
        h2r_s[cols, :] = h2.astype(BF16).T
        x_s[:, cols] = (x1 + lanes(col_s[3]) * h2).astype(BF16)
        rb = pltpu.bitcast(_rb(jnp.sum(h2 * lanes(col_s[4]), axis=0, keepdims=True)), I32)
        tok = i * TB + lax.broadcasted_iota(I32, (1, TB), 1)
        key = pltpu.bitcast(rb | jnp.where(rb >= 0, (S - 1) - tok, tok), F32)
        for u in range(TB // 128):
            key_s[pl.ds(i * (TB // 128) + u, 1), :] = key[:, u * 128:(u + 1) * 128]
        for u in range(TB // 128):
            out_copy(i * (TB // 128) + u).start()

    a_s[...] = o_proj(0, 0) + o_proj(0, 1)

    def p3_body(i, carry):
        a = a_s[...]
        a_s[...] = o_proj(i + 1, 0)
        resid_norm(i, a)
        a_s[...] += o_proj(i + 1, 1)
        return carry

    lax.fori_loop(0, ntb - 1, p3_body, 0)
    resid_norm(ntb - 1, a_s[...])

    sub = lax.broadcasted_iota(I32, (8, 128), 0)
    keyc = [key_s[g * 8:(g + 1) * 8, :] for g in range(S // 1024)]

    def token_row(ref, idx):
        word = ref[pl.ds(idx // 2, 1), :]
        bits = jnp.where(idx % 2 == 0, word << 16, word & jnp.int32(-65536))
        return pltpu.bitcast(jnp.broadcast_to(bits, (8, D)), F32)

    sub_d = lax.broadcasted_iota(I32, (8, D), 0)
    xsel = jnp.zeros((8, D), F32)
    best = jnp.zeros((8, 128), F32)
    idxs = []
    for j in range(TOPC):
        mx = functools.reduce(jnp.maximum, keyc)
        mx = jnp.max(jnp.max(mx, axis=0, keepdims=True), axis=1, keepdims=True)
        mxb = jnp.broadcast_to(mx, (8, 128))
        keyc = [jnp.where(kc == mxb, -jnp.inf, kc) for kc in keyc]
        best = jnp.where(sub == j, mxb, best)
        mb = pltpu.bitcast(mxb, I32)
        low = mb & (S - 1)
        idx = jnp.max(jnp.where(mb >= 0, (S - 1) - low, low))
        idxs.append(idx)
        xsel = jnp.where(sub_d == j, token_row(h2r_s.bitcast(I32), idx), xsel)

    rsel = pltpu.bitcast(pltpu.bitcast(best, I32) & jnp.int32(-65536), F32)[:, 0:1]
    xs = jnp.concatenate([xsel, xsel], axis=0).astype(BF16)
    g = _rb(jnp.dot(xs, wg_s[...], preferred_element_type=F32)[0:8])
    up = _rb(jnp.dot(xs, wu_s[...], preferred_element_type=F32)[0:8])
    act = _rb(_rb(g * _rb(jax.nn.sigmoid(g))) * up)
    act = jnp.concatenate([act, act], axis=0).astype(BF16)
    y = _rb(jnp.dot(act, wdt_s[...], preferred_element_type=F32)[0:8])
    y = _rb(y * _rb(jax.nn.sigmoid(rsel)))
    upd = gb * (_rb(xsel + y) - xsel)

    updt = jnp.concatenate([upd, jnp.zeros((120, D), F32)], axis=0).astype(BF16).T
    row16 = lax.broadcasted_iota(I32, (16, 128), 0)
    lane16 = lax.broadcasted_iota(I32, (16, 128), 1)
    idx_rows = jnp.full((16, 128), -1, I32)
    for j in range(TOPC):
        idx_rows = jnp.where(row16 == j, idxs[j], idx_rows)
    tiles = [idx // 128 for idx in idxs]

    def tile_copy(j):
        cols = pl.ds(pl.multiple_of(tiles[j] * 128, 128), 128)
        return pltpu.make_async_copy(patch_s.at[j], o_hbm.at[:, cols], sem_p.at[j])

    def first_in_tile(j):
        return functools.reduce(jnp.logical_and, [tiles[j] != tiles[i] for i in range(j)], True)

    for t in range(S // 128):
        out_copy(t).wait()
    for j in range(TOPC):
        onehot = (idx_rows - tiles[j] * 128 == lane16).astype(BF16)
        moved = jnp.dot(updt[:, 0:16], onehot, preferred_element_type=F32)
        old = x_s[:, pl.ds(pl.multiple_of(tiles[j] * 128, 128), 128)].astype(F32)
        patch_s[j] = (old + moved).astype(BF16)

        @pl.when(first_in_tile(j))
        def _():
            tile_copy(j).start()

    for j in range(TOPC):
        @pl.when(first_in_tile(j))
        def _():
            tile_copy(j).wait()


@jax.jit
def pallas_adaLN_cond__gqa_block_cached__moe_arch_mod__prompt_kernel(
    A_x: jax.Array,
    A_k_cache: jax.Array,
    A_v_cache: jax.Array,
    A_wq: jax.Array,
    A_wo: jax.Array,
    B_x: jax.Array,
    B_w_r: jax.Array,
    B_w_gate: jax.Array,
    B_w_up: jax.Array,
    B_w_down: jax.Array,
    c: jax.Array,
    w_mod: jax.Array,
):
    del B_x
    B, S, D = A_x.shape
    _, HKV, SK, DH = A_k_cache.shape
    HQ = A_wq.shape[1] // DH
    F = B_w_gate.shape[1]
    assert B == 1 and SK == S and DH == 128 and S % 1024 == 0 and S <= 65536

    vm = pltpu.VMEM
    dma = pltpu.SemaphoreType.DMA
    hbm = pl.BlockSpec(memory_space=pl.ANY)
    out = pl.pallas_call(
        functools.partial(_kernel, S=S, D=D, HQ=HQ, HKV=HKV, DH=DH, F=F),
        out_shape=jax.ShapeDtypeStruct((D, S), BF16),
        in_specs=[hbm] * 11,
        out_specs=hbm,
        scratch_shapes=[
            vm((D, S), BF16),
            vm((HKV, S, DH), BF16),
            vm((HKV, S, DH), BF16),
            vm((D, HQ * DH), BF16),
            vm((HQ, D, DH), BF16),
            vm((D, F), BF16),
            vm((D, F), BF16),
            vm((D, F), BF16),
            vm((D, 6 * D), BF16),
            vm((HQ, S, DH), BF16),
            vm((HQ, S, DH), BF16),
            vm((2, BQ, S), F32),
            vm((2, BQ, 128), F32),
            vm((2, -(-D // 128), RB, 128), BF16),
            vm((RB // 128, 128, D), F32),
            vm((2, 8, D), F32),
            vm((D, TB), F32),
            vm((5, D, 128), F32),
            vm((S, D), BF16),
            vm((S // 128, 128), F32),
            vm((F, D), BF16),
            vm((TOPC, D, 128), BF16),
            vm((1, D), BF16),
            vm((D,), BF16),
            dma((3,)), dma((len(WQ_GROUPS),)), dma((7 + HQ,)), dma((S // 128,)), dma((2,)), dma((TOPC,)),
            pltpu.SemaphoreType.REGULAR,
        ],
        compiler_params=pltpu.CompilerParams(
            vmem_limit_bytes=118 * 1024 * 1024,
            flags={"XLA_TPU_FORCE_LP_LLO_SCHEDULER": True},
        ),
        name="adaln_gqa_moe_block",
    )(c, B_w_r, A_x[0].T, A_k_cache[0], A_v_cache[0], A_wq, A_wo.T,
      B_w_gate, B_w_up, B_w_down.T, w_mod)
    return out.T[None]
```

```python
import functools

import jax
import jax.numpy as jnp
import jax.experimental.pallas as pl
import jax.experimental.pallas.tpu as pltpu
import numpy as np
from jax import lax

F32 = jnp.float32
BF16 = jnp.bfloat16
I32 = jnp.int32

NT_DIMS = (((1,), (1,)), ((), ()))
TOPC = 8
LN_EPS = 1e-5
LN_EPS_BF16 = float(np.asarray(LN_EPS, dtype=jnp.bfloat16))
LOG2E = 1.4426950408889634

RB = 512
BQ = 256
TB = 256
WQ_CHUNK = 512
WQ_GROUPS = (1, 2, 4, 1)


def _rb(a):
    return a.astype(BF16).astype(F32)


def _unpack(a):
    return pltpu.bitcast(a, BF16)


def _fold(a, op):
    out = a[:, :128]
    for j in range(1, a.shape[1] // 128):
        out = op(out, a[:, j * 128:(j + 1) * 128])
    return out


def _kernel(c_hbm, wr_hbm, x_hbm, k_hbm, v_hbm, wq_hbm, wo_hbm, wg_hbm, wu_hbm, wd_hbm,
            wmod_hbm, o_hbm,
            x_s, k_s, v_s, wq_s, wo_s, wg_s, wu_s, wd_s, wmod_s,
            q_s, o_s, s_s, m_s, h_s, xn_s, ms_s, a_s, col_s, h2r_s, wdt_s, patch_s,
            c_s, wr_s,
            sem_x, sem_wq, sem_w, sem_l, sem_o, sem_p, sem_f,
            *, S, D, HQ, HKV, DH, F):
    mod_a = 2 * D
    rep = HQ // HKV
    k_i = k_s.bitcast(I32)
    v_i = v_s.bitcast(I32)
    q_i = q_s.bitcast(I32)
    o_i = o_s.bitcast(I32)
    h_i = h_s.bitcast(I32)
    wo_i = wo_s.bitcast(I32)

    nrb = S // RB
    nwq = HQ * DH // WQ_CHUNK
    assert sum(WQ_GROUPS) == nwq and nrb >= 3
    g_lo = np.cumsum((0,) + WQ_GROUPS)

    def x_copy(g):
        cols = pl.ds(g * RB, RB if g < 2 else S - 2 * RB)
        return pltpu.make_async_copy(x_hbm.at[:, cols], x_s.at[:, cols], sem_x.at[g])

    def wq_copy(g):
        cols = pl.ds(int(g_lo[g]) * WQ_CHUNK, WQ_GROUPS[g] * WQ_CHUNK)
        return pltpu.make_async_copy(wq_hbm.at[:, cols], wq_s.at[:, cols], sem_wq.at[g])

    def out_copy(t):
        cols = pl.ds(pl.multiple_of(t * 128, 128), 128)
        return pltpu.make_async_copy(x_s.at[:, cols], o_hbm.at[:, cols], sem_o)

    moda_copy = pltpu.make_async_copy(
        wmod_hbm.at[:, pl.ds(0, mod_a)], wmod_s.at[:, pl.ds(0, mod_a)], sem_w.at[0])
    modb_copy = pltpu.make_async_copy(
        wmod_hbm.at[:, pl.ds(mod_a, 4 * D)], wmod_s.at[:, pl.ds(mod_a, 4 * D)], sem_w.at[1])
    c_copy = pltpu.make_async_copy(c_hbm, c_s, sem_w.at[4])
    wr_copy = pltpu.make_async_copy(wr_hbm, wr_s, sem_w.at[5])
    k_copy = pltpu.make_async_copy(k_hbm, k_s, sem_w.at[2])
    v_copy = pltpu.make_async_copy(v_hbm, v_s, sem_w.at[3])
    late_copies = [
        pltpu.make_async_copy(wg_hbm, wg_s, sem_l),
        pltpu.make_async_copy(wu_hbm, wu_s, sem_l),
        pltpu.make_async_copy(wd_hbm, wd_s, sem_l),
    ] + [
        pltpu.make_async_copy(wo_hbm.at[:, pl.ds(h * DH, DH)], wo_s.at[h], sem_l)
        for h in range(HQ)
    ]

    npan = -(-D // 128)
    qscale = (DH ** -0.5) * LOG2E

    def normalise(i, c):
        cols = pl.ds(pl.multiple_of(i * RB + c * 128, 128), 128)
        xv = x_s[:, cols].T.astype(F32)
        mean = jnp.sum(xv, axis=-1, keepdims=True) * (1.0 / D)
        xc = xv - mean
        var = jnp.sum(xc * xc, axis=-1, keepdims=True) * (1.0 / D)
        return xc * lax.rsqrt(var + LN_EPS)

    def put_h(slot, c, xn):
        hn = xn * jnp.tile(ms_s[0], (16, 1)) + jnp.tile(ms_s[1], (16, 1))
        if D % 128:
            hn = jnp.concatenate([hn, jnp.zeros((128, npan * 128 - D), F32)], axis=-1)
        for p in range(npan):
            h_s[slot, p, c * 128:(c + 1) * 128, :] = hn[:, p * 128:(p + 1) * 128].astype(BF16)

    def ln1(i, slot):
        for c in range(RB // 128):
            put_h(slot, c, normalise(i, c))

    def get_h(slot):
        pans = [_unpack(h_i[slot, p]) for p in range(npan)]
        return jnp.concatenate(pans, axis=-1)[:, 0:D]

    def q_proj(i, slot, before=None):
        for j in range(nwq):
            if before is not None:
                before(j)
            q = jnp.dot(get_h(slot), wq_s[:, j * WQ_CHUNK:(j + 1) * WQ_CHUNK],
                        preferred_element_type=F32)
            for u in range(WQ_CHUNK // DH):
                q_s[j * (WQ_CHUNK // DH) + u, pl.ds(pl.multiple_of(i * RB, RB), RB), :] = (
                    q[:, u * DH:(u + 1) * DH] * qscale).astype(BF16)

    def fence():
        pl.semaphore_signal(sem_f, 1)
        pl.semaphore_wait(sem_f, 1)

    for cp in (c_copy, x_copy(0), moda_copy, wq_copy(0), wq_copy(1), x_copy(1), wq_copy(2), wq_copy(3),
               x_copy(2), wr_copy, modb_copy, k_copy, v_copy):
        cp.start()
        fence()
    c_copy.wait()
    x_copy(0).wait()
    cv = c_s[...].astype(F32)
    sc = _rb(cv * _rb(jax.nn.sigmoid(cv)))
    sc = jnp.broadcast_to(sc, (16, D)).astype(BF16)
    for c in range(RB // 128):
        xn_s[c] = normalise(0, c)
    moda_copy.wait()
    mod = _rb(jnp.dot(sc, wmod_s[:, 0:mod_a], preferred_element_type=F32))[0:8]
    ms_s[0] = _rb(1.0 + mod[:, D:2 * D])
    ms_s[1] = mod[:, 0:D]
    fence()
    for c in range(RB // 128):
        put_h(0, c, xn_s[c])
        fence()

    def first_block(j):
        for g in range(len(WQ_GROUPS)):
            if j == g_lo[g]:
                wq_copy(g).wait()
                if g == 2:
                    x_copy(1).wait()
                    ln1(1, 1)

    q_proj(0, 0, first_block)
    x_copy(2).wait()

    def p1_body(i, carry):
        def mid(j):
            if j == nwq // 2:
                ln1(i + 1, (i + 1) & 1)

        q_proj(i, i & 1, mid)
        return carry

    lax.fori_loop(1, nrb - 1, p1_body, 0)

    wr_copy.wait()
    modb_copy.wait()
    k_copy.wait()
    v_copy.wait()
    for cp in late_copies:
        cp.start()
    mod2 = _rb(jnp.dot(sc, wmod_s[:, mod_a:6 * D], preferred_element_type=F32))[0:8]
    gb = mod2[:, 3 * D:4 * D]
    for n, row in enumerate((mod2[:, 0:D], mod2[:, D:2 * D], _rb(1.0 + mod2[:, 2 * D:3 * D]), gb,
                             wr_s[...].astype(F32).reshape(1, D))):
        col_s[n] = jnp.broadcast_to(row[0:1], (128, D)).T
    q_proj(nrb - 1, (nrb - 1) & 1)

    nbh = S // BQ
    nu = rep * nbh
    half = BQ // 2
    assert nu % 2 == 0

    def finish_max(slot):
        m = jnp.max(m_s[slot], axis=-1, keepdims=True)
        m_s[slot] = jnp.broadcast_to(m, (BQ, 128))

    def qk(h, u, defer):
        slot = u % 2
        q = _unpack(q_i[h * rep + u // nbh, (u % nbh) * half:(u % nbh + 1) * half, :])
        s = lax.dot_general(q, _unpack(k_i[h]), NT_DIMS, preferred_element_type=F32)
        s_s[slot] = s
        m_s[slot] = _fold(s, jnp.maximum)
        if not defer:
            finish_max(slot)

    def pv(h, u):
        slot = u % 2
        p = jnp.exp2(s_s[slot] - jnp.tile(m_s[slot], (1, S // 128)))
        l = jnp.sum(_fold(p, jnp.add), axis=-1, keepdims=True)
        acc = jnp.dot(p.astype(BF16), _unpack(v_i[h]), preferred_element_type=F32)
        inv = pl.reciprocal(l, approx=True)
        inv = inv * (2.0 - l * inv)
        o_s[h * rep + u // nbh, (u % nbh) * BQ:(u % nbh + 1) * BQ, :] = (acc * inv).astype(BF16)

    def p2_head(h, last):
        finish_max(1)
        for u in range(nu):
            pv(h, u)
            if u + 2 < nu:
                qk(h, u + 2, False)
            elif not last:
                qk(h + 1, u + 2 - nu, u == nu - 1)

    qk(0, 0, False)
    qk(0, 1, True)

    def p2_body(h, carry):
        p2_head(h, False)
        return carry

    lax.fori_loop(0, HKV - 1, p2_body, 0)
    for cp in late_copies:
        cp.wait()
    for j in range(F // 128):
        wdt_s[j * 128:(j + 1) * 128, :] = wd_s[:, j * 128:(j + 1) * 128].T
    p2_head(HKV - 1, True)

    ntb = S // TB
    lanes = lambda a: jnp.tile(a, (1, TB // 128))

    def o_proj(i, kh):
        rows = pl.ds(pl.multiple_of(i * (TB // 2), TB // 2), TB // 2)
        h0, h1 = kh * HQ // 2, (kh + 1) * HQ // 2
        ob = jnp.concatenate([_unpack(o_i[h, rows, :]) for h in range(h0, h1)], axis=-1)
        wt = jnp.concatenate([_unpack(wo_i[h]) for h in range(h0, h1)], axis=-1)
        return lax.dot_general(wt, ob, NT_DIMS, preferred_element_type=F32)

    def resid_norm(i, a):
        cols = pl.ds(pl.multiple_of(i * TB, TB), TB)
        x1 = _rb(x_s[:, cols].astype(F32) + lanes(col_s[0]) * a)
        mean = jnp.sum(x1, axis=0, keepdims=True) * (1.0 / D)
        xc = x1 - mean
        var = jnp.sum(xc * xc, axis=0, keepdims=True) * (1.0 / D)
        std = _rb(jnp.sqrt(_rb(_rb(var) + LN_EPS_BF16)))
        hn = _rb(_rb(x1 - _rb(mean)) / std)
        h2 = _rb(_rb(hn * lanes(col_s[2])) + lanes(col_s[1]))
        h2r_s[cols, :] = h2.astype(BF16).T
        x_s[:, cols] = (x1 + lanes(col_s[3]) * h2).astype(BF16)
        rb = pltpu.bitcast(_rb(jnp.sum(h2 * lanes(col_s[4]), axis=0, keepdims=True)), I32)
        tok = i * TB + lax.broadcasted_iota(I32, (1, TB), 1)
        key = pltpu.bitcast(rb | jnp.where(rb >= 0, (S - 1) - tok, tok), F32)
        kb = jnp.full((8, 128), -jnp.inf, F32)
        for u in range(TB // 128):
            kb = jnp.where(sub == u, key[:, u * 128:(u + 1) * 128], kb)
        for u in range(TB // 128):
            out_copy(i * (TB // 128) + u).start()
        return kb

    sub = lax.broadcasted_iota(I32, (8, 128), 0)

    def max_all(a):
        m = jnp.max(jnp.max(a, axis=0, keepdims=True), axis=1, keepdims=True)
        return jnp.broadcast_to(m, (8, 128))

    def merge_top(top, kb):
        out = top
        for j in range(TOPC):
            m = max_all(jnp.maximum(top, kb))
            top = jnp.where(top == m, -jnp.inf, top)
            kb = jnp.where(kb == m, -jnp.inf, kb)
            out = jnp.where(sub == j, m, out)
        return out

    a_s[...] = o_proj(0, 0) + o_proj(0, 1)

    def p3_body(i, top):
        a = a_s[...]
        a_s[...] = o_proj(i + 1, 0)
        kb = resid_norm(i, a)
        a_s[...] += o_proj(i + 1, 1)
        return merge_top(top, kb)

    assert TOPC == 8 and TB // 128 <= 8 and S - TB >= TOPC
    top = lax.fori_loop(0, ntb - 1, p3_body, jnp.full((8, 128), -jnp.inf, F32))
    kb = resid_norm(ntb - 1, a_s[...])

    def more(state):
        top, kb, best = state
        return jnp.max(jnp.where(best > jnp.min(top, axis=0, keepdims=True), 1, 0)) > 0

    def insert(state):
        top, kb, best = state
        top = jnp.where(top == jnp.min(top, axis=0, keepdims=True), best, top)
        kb = jnp.where(kb == best, -jnp.inf, kb)
        return top, kb, max_all(kb)

    top, _, _ = lax.while_loop(more, insert, (top, kb, max_all(kb)))

    def token_row(ref, idx):
        word = ref[pl.ds(idx // 2, 1), :]
        bits = jnp.where(idx % 2 == 0, word << 16, word & jnp.int32(-65536))
        return pltpu.bitcast(jnp.broadcast_to(bits, (8, D)), F32)

    sub_d = lax.broadcasted_iota(I32, (8, D), 0)
    xsel = jnp.zeros((8, D), F32)
    top_bits = pltpu.bitcast(top, I32)
    low = top_bits & (S - 1)
    tok = jnp.where(top_bits >= 0, (S - 1) - low, low)
    idxs = []
    for j in range(TOPC):
        idx = jnp.max(jnp.where(sub == j, tok, 0))
        idxs.append(idx)
        xsel = jnp.where(sub_d == j, token_row(h2r_s.bitcast(I32), idx), xsel)

    rsel = pltpu.bitcast(top_bits & jnp.int32(-65536), F32)[:, 0:1]
    xs = jnp.concatenate([xsel, xsel], axis=0).astype(BF16)
    g = _rb(jnp.dot(xs, wg_s[...], preferred_element_type=F32)[0:8])
    up = _rb(jnp.dot(xs, wu_s[...], preferred_element_type=F32)[0:8])
    act = _rb(_rb(g * _rb(jax.nn.sigmoid(g))) * up)
    act = jnp.concatenate([act, act], axis=0).astype(BF16)
    y = _rb(jnp.dot(act, wdt_s[...], preferred_element_type=F32)[0:8])
    y = _rb(y * _rb(jax.nn.sigmoid(rsel)))
    upd = gb * (_rb(xsel + y) - xsel)

    updt = jnp.concatenate([upd, jnp.zeros((8, D), F32)], axis=0).astype(BF16).T
    row16 = lax.broadcasted_iota(I32, (16, 128), 0)
    lane16 = lax.broadcasted_iota(I32, (16, 128), 1)
    idx_rows = jnp.full((16, 128), -1, I32)
    for j in range(TOPC):
        idx_rows = jnp.where(row16 == j, idxs[j], idx_rows)
    tiles = [idx // 128 for idx in idxs]

    def tile_copy(j):
        cols = pl.ds(pl.multiple_of(tiles[j] * 128, 128), 128)
        return pltpu.make_async_copy(patch_s.at[j], o_hbm.at[:, cols], sem_p)

    def first_in_tile(j):
        return functools.reduce(jnp.logical_and, [tiles[j] != tiles[i] for i in range(j)], True)

    for t in range(S // 128):
        out_copy(t).wait()
    for j in range(TOPC):
        onehot = (idx_rows - tiles[j] * 128 == lane16).astype(BF16)
        moved = jnp.dot(updt, onehot, preferred_element_type=F32)
        old = x_s[:, pl.ds(pl.multiple_of(tiles[j] * 128, 128), 128)].astype(F32)
        patch_s[j] = (old + moved).astype(BF16)

        @pl.when(first_in_tile(j))
        def _():
            tile_copy(j).start()

    for j in range(TOPC):
        @pl.when(first_in_tile(j))
        def _():
            tile_copy(j).wait()


@jax.jit
def pallas_adaLN_cond__gqa_block_cached__moe_arch_mod__prompt_kernel(
    A_x: jax.Array,
    A_k_cache: jax.Array,
    A_v_cache: jax.Array,
    A_wq: jax.Array,
    A_wo: jax.Array,
    B_x: jax.Array,
    B_w_r: jax.Array,
    B_w_gate: jax.Array,
    B_w_up: jax.Array,
    B_w_down: jax.Array,
    c: jax.Array,
    w_mod: jax.Array,
):
    del B_x
    B, S, D = A_x.shape
    _, HKV, SK, DH = A_k_cache.shape
    HQ = A_wq.shape[1] // DH
    F = B_w_gate.shape[1]
    assert B == 1 and SK == S and DH == 128 and S % 1024 == 0 and S <= 65536

    vm = pltpu.VMEM
    dma = pltpu.SemaphoreType.DMA
    hbm = pl.BlockSpec(memory_space=pl.ANY)
    out = pl.pallas_call(
        functools.partial(_kernel, S=S, D=D, HQ=HQ, HKV=HKV, DH=DH, F=F),
        out_shape=jax.ShapeDtypeStruct((D, S), BF16),
        in_specs=[hbm] * 11,
        out_specs=hbm,
        scratch_shapes=[
            vm((D, S), BF16),
            vm((HKV, S, DH), BF16),
            vm((HKV, S, DH), BF16),
            vm((D, HQ * DH), BF16),
            vm((HQ, D, DH), BF16),
            vm((D, F), BF16),
            vm((D, F), BF16),
            vm((D, F), BF16),
            vm((D, 6 * D), BF16),
            vm((HQ, S, DH), BF16),
            vm((HQ, S, DH), BF16),
            vm((2, BQ, S), F32),
            vm((2, BQ, 128), F32),
            vm((2, -(-D // 128), RB, 128), BF16),
            vm((RB // 128, 128, D), F32),
            vm((2, 8, D), F32),
            vm((D, TB), F32),
            vm((5, D, 128), F32),
            vm((S, D), BF16),
            vm((F, D), BF16),
            vm((TOPC, D, 128), BF16),
            vm((1, D), BF16),
            vm((D,), BF16),
            dma((3,)), dma((len(WQ_GROUPS),)), dma((6,)), dma, dma, dma,
            pltpu.SemaphoreType.REGULAR,
        ],
        compiler_params=pltpu.CompilerParams(
            vmem_limit_bytes=118 * 1024 * 1024,
            flags={"XLA_TPU_FORCE_LP_LLO_SCHEDULER": True},
        ),
        name="adaln_gqa_moe_block",
    )(c, B_w_r, A_x[0].T, A_k_cache[0], A_v_cache[0], A_wq, A_wo.T,
      B_w_gate, B_w_up, B_w_down.T, w_mod)
    return out.T[None]
```

```python
import functools

import jax
import jax.numpy as jnp
import jax.experimental.pallas as pl
import jax.experimental.pallas.tpu as pltpu
import numpy as np
from jax import lax

F32 = jnp.float32
BF16 = jnp.bfloat16
I32 = jnp.int32

NT_DIMS = (((1,), (1,)), ((), ()))
TOPC = 8
LN_EPS = 1e-5
LN_EPS_BF16 = float(np.asarray(LN_EPS, dtype=jnp.bfloat16))
LOG2E = 1.4426950408889634

RB = 512
BQ = 256
TB = 256
WQ_CHUNK = 512
WQ_GROUPS = (1, 2, 4, 1)


def _rb(a):
    return a.astype(BF16).astype(F32)


def _unpack(a):
    return pltpu.bitcast(a, BF16)


def _fold(a, op):
    out = a[:, :128]
    for j in range(1, a.shape[1] // 128):
        out = op(out, a[:, j * 128:(j + 1) * 128])
    return out


def _kernel(c_hbm, wr_hbm, x_hbm, k_hbm, v_hbm, wq_hbm, wo_hbm, wg_hbm, wu_hbm, wd_hbm,
            wmod_hbm, o_hbm,
            x_s, k_s, v_s, wq_s, wo_s, wg_s, wu_s, wd_s, wmod_s,
            q_s, o_s, s_s, m_s, h_s, xn_s, ms_s, a_s, col_s, h2r_s, wdt_s, patch_s,
            c_s, wr_s,
            sem_x, sem_wq, sem_w, sem_l, sem_o, sem_p, sem_f,
            *, S, D, HQ, HKV, DH, F):
    mod_a = 2 * D
    rep = HQ // HKV
    k_i = k_s.bitcast(I32)
    v_i = v_s.bitcast(I32)
    q_i = q_s.bitcast(I32)
    o_i = o_s.bitcast(I32)
    h_i = h_s.bitcast(I32)
    wo_i = wo_s.bitcast(I32)

    nrb = S // RB
    nwq = HQ * DH // WQ_CHUNK
    assert sum(WQ_GROUPS) == nwq and nrb >= 3 and nwq == 2 * (RB // 128)
    g_lo = np.cumsum((0,) + WQ_GROUPS)

    def x_copy(g):
        cols = pl.ds(g * RB, RB if g < 2 else S - 2 * RB)
        return pltpu.make_async_copy(x_hbm.at[:, cols], x_s.at[:, cols], sem_x.at[g])

    def wq_copy(g):
        cols = pl.ds(int(g_lo[g]) * WQ_CHUNK, WQ_GROUPS[g] * WQ_CHUNK)
        return pltpu.make_async_copy(wq_hbm.at[:, cols], wq_s.at[:, cols], sem_wq.at[g])

    def out_copy(t):
        cols = pl.ds(pl.multiple_of(t * 128, 128), 128)
        return pltpu.make_async_copy(x_s.at[:, cols], o_hbm.at[:, cols], sem_o)

    moda_copy = pltpu.make_async_copy(
        wmod_hbm.at[:, pl.ds(0, mod_a)], wmod_s.at[:, pl.ds(0, mod_a)], sem_w.at[0])
    modb_copy = pltpu.make_async_copy(
        wmod_hbm.at[:, pl.ds(mod_a, 4 * D)], wmod_s.at[:, pl.ds(mod_a, 4 * D)], sem_w.at[1])
    c_copy = pltpu.make_async_copy(c_hbm, c_s, sem_w.at[4])
    wr_copy = pltpu.make_async_copy(wr_hbm, wr_s, sem_w.at[5])
    k_copy = pltpu.make_async_copy(k_hbm, k_s, sem_w.at[2])
    v_copy = pltpu.make_async_copy(v_hbm, v_s, sem_w.at[3])
    late_copies = [
        pltpu.make_async_copy(wg_hbm, wg_s, sem_l),
        pltpu.make_async_copy(wu_hbm, wu_s, sem_l),
        pltpu.make_async_copy(wd_hbm, wd_s, sem_l),
    ] + [
        pltpu.make_async_copy(wo_hbm.at[:, pl.ds(h * DH, DH)], wo_s.at[h], sem_l)
        for h in range(HQ)
    ]

    npan = -(-D // 128)
    qscale = (DH ** -0.5) * LOG2E

    def normalise(i, c):
        cols = pl.ds(pl.multiple_of(i * RB + c * 128, 128), 128)
        xv = x_s[:, cols].T.astype(F32)
        mean = jnp.sum(xv, axis=-1, keepdims=True) * (1.0 / D)
        xc = xv - mean
        var = jnp.sum(xc * xc, axis=-1, keepdims=True) * (1.0 / D)
        return xc * lax.rsqrt(var + LN_EPS)

    def put_h(slot, c, xn):
        hn = xn * jnp.tile(ms_s[0], (16, 1)) + jnp.tile(ms_s[1], (16, 1))
        if D % 128:
            hn = jnp.concatenate([hn, jnp.zeros((128, npan * 128 - D), F32)], axis=-1)
        for p in range(npan):
            h_s[slot, p, c * 128:(c + 1) * 128, :] = hn[:, p * 128:(p + 1) * 128].astype(BF16)

    def get_h(slot):
        pans = [_unpack(h_i[slot, p]) for p in range(npan)]
        return jnp.concatenate(pans, axis=-1)[:, 0:D]

    def q_proj(i, slot, before=None):
        for j in range(nwq):
            if before is not None:
                before(j)
            q = jnp.dot(get_h(slot), wq_s[:, j * WQ_CHUNK:(j + 1) * WQ_CHUNK],
                        preferred_element_type=F32)
            for u in range(WQ_CHUNK // DH):
                q_s[j * (WQ_CHUNK // DH) + u, pl.ds(pl.multiple_of(i * RB, RB), RB), :] = (
                    q[:, u * DH:(u + 1) * DH] * qscale).astype(BF16)

    def fence():
        pl.semaphore_signal(sem_f, 1)
        pl.semaphore_wait(sem_f, 1)

    for cp in (c_copy, x_copy(0), moda_copy, wq_copy(0), wq_copy(1), x_copy(1), wq_copy(2), wq_copy(3),
               x_copy(2), wr_copy, modb_copy, k_copy, v_copy):
        cp.start()
        fence()
    c_copy.wait()
    x_copy(0).wait()
    cv = c_s[...].astype(F32)
    sc = _rb(cv * _rb(jax.nn.sigmoid(cv)))
    sc = jnp.broadcast_to(sc, (16, D)).astype(BF16)
    for c in range(RB // 128):
        xn_s[c] = normalise(0, c)
    moda_copy.wait()
    mod = _rb(jnp.dot(sc, wmod_s[:, 0:mod_a], preferred_element_type=F32))[0:8]
    ms_s[0] = _rb(1.0 + mod[:, D:2 * D])
    ms_s[1] = mod[:, 0:D]
    fence()
    for c in range(RB // 128):
        put_h(0, c, xn_s[c])
        fence()

    def first_block(j):
        for g in range(len(WQ_GROUPS)):
            if j == g_lo[g]:
                wq_copy(g).wait()
                if g == 2:
                    x_copy(1).wait()
        c = j - (nwq - RB // 128)
        if c >= 0:
            put_h(1, c, normalise(1, c))

    q_proj(0, 0, first_block)
    x_copy(2).wait()

    def p1_body(i, carry):
        def mid(j):
            if j % 2:
                c = j // 2
                put_h((i + 1) & 1, c, normalise(i + 1, c))

        q_proj(i, i & 1, mid)
        return carry

    lax.fori_loop(1, nrb - 1, p1_body, 0)

    wr_copy.wait()
    modb_copy.wait()
    k_copy.wait()
    v_copy.wait()
    for cp in late_copies:
        cp.start()
    mod2 = _rb(jnp.dot(sc, wmod_s[:, mod_a:6 * D], preferred_element_type=F32))[0:8]
    gb = mod2[:, 3 * D:4 * D]
    for n, row in enumerate((mod2[:, 0:D], mod2[:, D:2 * D], _rb(1.0 + mod2[:, 2 * D:3 * D]), gb,
                             wr_s[...].astype(F32).reshape(1, D))):
        col_s[n] = jnp.broadcast_to(row[0:1], (128, D)).T
    q_proj(nrb - 1, (nrb - 1) & 1)

    nbh = S // BQ
    nu = rep * nbh
    half = BQ // 2
    assert nu % 2 == 0

    def finish_max(slot):
        m = jnp.max(m_s[slot], axis=-1, keepdims=True)
        m_s[slot] = jnp.broadcast_to(m, (BQ, 128))

    def qk(h, u, defer):
        slot = u % 2
        q = _unpack(q_i[h * rep + u // nbh, (u % nbh) * half:(u % nbh + 1) * half, :])
        s = lax.dot_general(q, _unpack(k_i[h]), NT_DIMS, preferred_element_type=F32)
        s_s[slot] = s
        m_s[slot] = _fold(s, jnp.maximum)
        if not defer:
            finish_max(slot)

    def pv(h, u):
        slot = u % 2
        p = jnp.exp2(s_s[slot] - jnp.tile(m_s[slot], (1, S // 128)))
        l = jnp.sum(_fold(p, jnp.add), axis=-1, keepdims=True)
        acc = jnp.dot(p.astype(BF16), _unpack(v_i[h]), preferred_element_type=F32)
        inv = pl.reciprocal(l, approx=True)
        inv = inv * (2.0 - l * inv)
        o_s[h * rep + u // nbh, (u % nbh) * BQ:(u % nbh + 1) * BQ, :] = (acc * inv).astype(BF16)

    def p2_head(h, last):
        finish_max(1)
        for u in range(nu):
            pv(h, u)
            if u + 2 < nu:
                qk(h, u + 2, False)
            elif not last:
                qk(h + 1, u + 2 - nu, u == nu - 1)

    qk(0, 0, False)
    qk(0, 1, True)

    def p2_body(h, carry):
        p2_head(h, False)
        return carry

    lax.fori_loop(0, HKV - 1, p2_body, 0)
    for cp in late_copies:
        cp.wait()
    for j in range(F // 128):
        wdt_s[j * 128:(j + 1) * 128, :] = wd_s[:, j * 128:(j + 1) * 128].T
    p2_head(HKV - 1, True)

    ntb = S // TB
    def o_proj(t0, n, kh=None):
        rows = pl.ds(pl.multiple_of(t0 // 2, 64), n // 2)
        h0, h1 = (0, HQ) if kh is None else (kh * HQ // 2, (kh + 1) * HQ // 2)
        ob = jnp.concatenate([_unpack(o_i[h, rows, :]) for h in range(h0, h1)], axis=-1)
        wt = jnp.concatenate([_unpack(wo_i[h]) for h in range(h0, h1)], axis=-1)
        return lax.dot_general(wt, ob, NT_DIMS, preferred_element_type=F32)

    def resid_norm(t0, n, a):
        cols = pl.ds(pl.multiple_of(t0, 128), n)
        lanes = lambda v: jnp.tile(v, (1, n // 128))
        x1 = _rb(x_s[:, cols].astype(F32) + lanes(col_s[0]) * a)
        mean = jnp.sum(x1, axis=0, keepdims=True) * (1.0 / D)
        xc = x1 - mean
        var = jnp.sum(xc * xc, axis=0, keepdims=True) * (1.0 / D)
        std = _rb(jnp.sqrt(_rb(_rb(var) + LN_EPS_BF16)))
        hn = _rb(_rb(x1 - _rb(mean)) / std)
        h2 = _rb(_rb(hn * lanes(col_s[2])) + lanes(col_s[1]))
        h2r_s[cols, :] = h2.astype(BF16).T
        x_s[:, cols] = (x1 + lanes(col_s[3]) * h2).astype(BF16)
        rb = pltpu.bitcast(_rb(jnp.sum(h2 * lanes(col_s[4]), axis=0, keepdims=True)), I32)
        tok = t0 + lax.broadcasted_iota(I32, (1, n), 1)
        key = pltpu.bitcast(rb | jnp.where(rb >= 0, (S - 1) - tok, tok), F32)
        kb = jnp.full((8, 128), -jnp.inf, F32)
        for u in range(n // 128):
            kb = jnp.where(sub == u, key[:, u * 128:(u + 1) * 128], kb)
        for u in range(n // 128):
            out_copy(t0 // 128 + u).start()
        return kb

    sub = lax.broadcasted_iota(I32, (8, 128), 0)

    def max_all(a):
        m = jnp.max(jnp.max(a, axis=0, keepdims=True), axis=1, keepdims=True)
        return jnp.broadcast_to(m, (8, 128))

    def merge_top(top, kb):
        out = top
        for j in range(TOPC):
            m = max_all(jnp.maximum(top, kb))
            top = jnp.where(top == m, -jnp.inf, top)
            kb = jnp.where(kb == m, -jnp.inf, kb)
            out = jnp.where(sub == j, m, out)
        return out

    a0 = o_proj(0, 128)
    a_s[:, 128:] = o_proj(128, 128)
    k00 = resid_norm(0, 128, a0)

    def p3_body(i, top):
        b = a_s[:, 128:]
        an = o_proj((i + 1) * TB, 128)
        k0 = resid_norm(i * TB + 128, 128, b)
        a_s[:, 128:] = o_proj((i + 1) * TB + 128, 128)
        k1 = resid_norm((i + 1) * TB, 128, an)
        return merge_top(merge_top(top, k0), k1)

    assert TOPC == 8 and TB // 128 <= 8 and S - TB >= TOPC
    top = lax.fori_loop(0, ntb - 1, p3_body, merge_top(jnp.full((8, 128), -jnp.inf, F32), k00))
    kb = resid_norm(S - 128, 128, a_s[:, 128:])

    def more(state):
        top, kb, best = state
        return jnp.max(jnp.where(best > jnp.min(top, axis=0, keepdims=True), 1, 0)) > 0

    def insert(state):
        top, kb, best = state
        top = jnp.where(top == jnp.min(top, axis=0, keepdims=True), best, top)
        kb = jnp.where(kb == best, -jnp.inf, kb)
        return top, kb, max_all(kb)

    top, _, _ = lax.while_loop(more, insert, (top, kb, max_all(kb)))

    def token_row(ref, idx):
        word = ref[pl.ds(lax.shift_right_logical(idx, 1), 1), :]
        bits = jnp.where((idx & 1) == 0, word << 16, word & jnp.int32(-65536))
        return pltpu.bitcast(jnp.broadcast_to(bits, (8, D)), F32)

    sub_d = lax.broadcasted_iota(I32, (8, D), 0)
    xsel = jnp.zeros((8, D), F32)
    top_bits = pltpu.bitcast(top, I32)
    low = top_bits & (S - 1)
    tok = jnp.where(top_bits >= 0, (S - 1) - low, low)
    idxs = []
    for j in range(TOPC):
        idx = jnp.max(jnp.where(sub == j, tok, 0))
        idxs.append(idx)
        xsel = jnp.where(sub_d == j, token_row(h2r_s.bitcast(I32), idx), xsel)

    rsel = pltpu.bitcast(top_bits & jnp.int32(-65536), F32)[:, 0:1]
    xs = jnp.concatenate([xsel, xsel], axis=0).astype(BF16)
    g = _rb(jnp.dot(xs, wg_s[...], preferred_element_type=F32)[0:8])
    up = _rb(jnp.dot(xs, wu_s[...], preferred_element_type=F32)[0:8])
    act = _rb(_rb(g * _rb(jax.nn.sigmoid(g))) * up)
    act = jnp.concatenate([act, act], axis=0).astype(BF16)
    y = _rb(jnp.dot(act, wdt_s[...], preferred_element_type=F32)[0:8])
    y = _rb(y * _rb(jax.nn.sigmoid(rsel)))
    upd = gb * (_rb(xsel + y) - xsel)

    updt = jnp.concatenate([upd, jnp.zeros((8, D), F32)], axis=0).astype(BF16).T
    row16 = lax.broadcasted_iota(I32, (16, 128), 0)
    lane16 = lax.broadcasted_iota(I32, (16, 128), 1)
    idx_rows = jnp.full((16, 128), -1, I32)
    for j in range(TOPC):
        idx_rows = jnp.where(row16 == j, idxs[j], idx_rows)
    tiles = [lax.shift_right_logical(idx, 7) for idx in idxs]

    def tile_copy(j):
        cols = pl.ds(pl.multiple_of(tiles[j] * 128, 128), 128)
        return pltpu.make_async_copy(patch_s.at[j], o_hbm.at[:, cols], sem_p)

    def first_in_tile(j):
        return functools.reduce(jnp.logical_and, [tiles[j] != tiles[i] for i in range(j)], True)

    for t in range(S // 128):
        out_copy(t).wait()
    for j in range(TOPC):
        onehot = (idx_rows - tiles[j] * 128 == lane16).astype(BF16)
        moved = jnp.dot(updt, onehot, preferred_element_type=F32)
        old = x_s[:, pl.ds(pl.multiple_of(tiles[j] * 128, 128), 128)].astype(F32)
        patch_s[j] = (old + moved).astype(BF16)

        @pl.when(first_in_tile(j))
        def _():
            tile_copy(j).start()

    for j in range(TOPC):
        @pl.when(first_in_tile(j))
        def _():
            tile_copy(j).wait()


@jax.jit
def pallas_adaLN_cond__gqa_block_cached__moe_arch_mod__prompt_kernel(
    A_x: jax.Array,
    A_k_cache: jax.Array,
    A_v_cache: jax.Array,
    A_wq: jax.Array,
    A_wo: jax.Array,
    B_x: jax.Array,
    B_w_r: jax.Array,
    B_w_gate: jax.Array,
    B_w_up: jax.Array,
    B_w_down: jax.Array,
    c: jax.Array,
    w_mod: jax.Array,
):
    del B_x
    B, S, D = A_x.shape
    _, HKV, SK, DH = A_k_cache.shape
    HQ = A_wq.shape[1] // DH
    F = B_w_gate.shape[1]
    assert B == 1 and SK == S and DH == 128 and S % 1024 == 0 and S <= 65536

    vm = pltpu.VMEM
    dma = pltpu.SemaphoreType.DMA
    hbm = pl.BlockSpec(memory_space=pl.ANY)
    out = pl.pallas_call(
        functools.partial(_kernel, S=S, D=D, HQ=HQ, HKV=HKV, DH=DH, F=F),
        out_shape=jax.ShapeDtypeStruct((D, S), BF16),
        in_specs=[hbm] * 11,
        out_specs=hbm,
        scratch_shapes=[
            vm((D, S), BF16),
            vm((HKV, S, DH), BF16),
            vm((HKV, S, DH), BF16),
            vm((D, HQ * DH), BF16),
            vm((HQ, D, DH), BF16),
            vm((D, F), BF16),
            vm((D, F), BF16),
            vm((D, F), BF16),
            vm((D, 6 * D), BF16),
            vm((HQ, S, DH), BF16),
            vm((HQ, S, DH), BF16),
            vm((2, BQ, S), F32),
            vm((2, BQ, 128), F32),
            vm((2, -(-D // 128), RB, 128), BF16),
            vm((RB // 128, 128, D), F32),
            vm((2, 8, D), F32),
            vm((D, TB), F32),
            vm((5, D, 128), F32),
            vm((S, D), BF16),
            vm((F, D), BF16),
            vm((TOPC, D, 128), BF16),
            vm((1, D), BF16),
            vm((D,), BF16),
            dma((3,)), dma((len(WQ_GROUPS),)), dma((6,)), dma, dma, dma,
            pltpu.SemaphoreType.REGULAR,
        ],
        compiler_params=pltpu.CompilerParams(
            vmem_limit_bytes=118 * 1024 * 1024,
            flags={"XLA_TPU_FORCE_LP_LLO_SCHEDULER": True},
        ),
        name="adaln_gqa_moe_block",
    )(c, B_w_r, A_x[0].T, A_k_cache[0], A_v_cache[0], A_wq, A_wo.T,
      B_w_gate, B_w_up, B_w_down.T, w_mod)
    return out.T[None]
```

```python
import functools

import jax
import jax.numpy as jnp
import jax.experimental.pallas as pl
import jax.experimental.pallas.tpu as pltpu
import numpy as np
from jax import lax

F32 = jnp.float32
BF16 = jnp.bfloat16
I32 = jnp.int32

NT_DIMS = (((1,), (1,)), ((), ()))
TOPC = 8
LN_EPS = 1e-5
LN_EPS_BF16 = float(np.asarray(LN_EPS, dtype=jnp.bfloat16))
LOG2E = 1.4426950408889634

RB = 512
BQ = 256
WQ_CHUNK = 512
WQ_GROUPS = (1, 2, 4, 1)


def _rb(a):
    return a.astype(BF16).astype(F32)


def _unpack(a):
    return pltpu.bitcast(a, BF16)


def _fold(a, op):
    out = a[:, :128]
    for j in range(1, a.shape[1] // 128):
        out = op(out, a[:, j * 128:(j + 1) * 128])
    return out


def _kernel(c_hbm, wr_hbm, x_hbm, k_hbm, v_hbm, wq_hbm, wo_hbm, wg_hbm, wu_hbm, wd_hbm,
            wmod_hbm, o_hbm,
            x_s, k_s, v_s, wq_s, wo_s, wg_s, wu_s, wd_s, wmod_s,
            q_s, o_s, s_s, m_s, h_s, xn_s, ms_s, col_s, h2r_s, wdt_s, patch_s,
            c_s, wr_s,
            sem_x, sem_wq, sem_w, sem_l, sem_o, sem_p, sem_f,
            *, S, D, HQ, HKV, DH, F):
    mod_a = 2 * D
    rep = HQ // HKV
    k_i = k_s.bitcast(I32)
    v_i = v_s.bitcast(I32)
    q_i = q_s.bitcast(I32)
    o_i = o_s.bitcast(I32)
    h_i = h_s.bitcast(I32)
    wo_i = wo_s.bitcast(I32)

    nrb = S // RB
    nwq = HQ * DH // WQ_CHUNK
    assert sum(WQ_GROUPS) == nwq and nrb >= 3 and nwq == 2 * (RB // 128)
    g_lo = np.cumsum((0,) + WQ_GROUPS)

    def x_copy(g):
        cols = pl.ds(g * RB, RB if g < 2 else S - 2 * RB)
        return pltpu.make_async_copy(x_hbm.at[:, cols], x_s.at[:, cols], sem_x.at[g])

    def wq_copy(g):
        cols = pl.ds(int(g_lo[g]) * WQ_CHUNK, WQ_GROUPS[g] * WQ_CHUNK)
        return pltpu.make_async_copy(wq_hbm.at[:, cols], wq_s.at[:, cols], sem_wq.at[g])

    def out_copy(t):
        cols = pl.ds(pl.multiple_of(t * 128, 128), 128)
        return pltpu.make_async_copy(x_s.at[:, cols], o_hbm.at[:, cols], sem_o)

    moda_copy = pltpu.make_async_copy(
        wmod_hbm.at[:, pl.ds(0, mod_a)], wmod_s.at[:, pl.ds(0, mod_a)], sem_w.at[0])
    modb_copy = pltpu.make_async_copy(
        wmod_hbm.at[:, pl.ds(mod_a, 4 * D)], wmod_s.at[:, pl.ds(mod_a, 4 * D)], sem_w.at[1])
    c_copy = pltpu.make_async_copy(c_hbm, c_s, sem_w.at[4])
    wr_copy = pltpu.make_async_copy(wr_hbm, wr_s, sem_w.at[5])
    k_copy = pltpu.make_async_copy(k_hbm, k_s, sem_w.at[2])
    v_copy = pltpu.make_async_copy(v_hbm, v_s, sem_w.at[3])
    late_copies = [
        pltpu.make_async_copy(wg_hbm, wg_s, sem_l),
        pltpu.make_async_copy(wu_hbm, wu_s, sem_l),
        pltpu.make_async_copy(wd_hbm, wd_s, sem_l),
    ] + [
        pltpu.make_async_copy(wo_hbm.at[:, pl.ds(h * DH, DH)], wo_s.at[h], sem_l)
        for h in range(HQ)
    ]

    npan = -(-D // 128)
    qscale = (DH ** -0.5) * LOG2E

    def normalise(i, c):
        cols = pl.ds(pl.multiple_of(i * RB + c * 128, 128), 128)
        xv = x_s[:, cols].T.astype(F32)
        mean = jnp.sum(xv, axis=-1, keepdims=True) * (1.0 / D)
        xc = xv - mean
        var = jnp.sum(xc * xc, axis=-1, keepdims=True) * (1.0 / D)
        return xc * lax.rsqrt(var + LN_EPS)

    def put_h(slot, c, xn):
        hn = xn * jnp.tile(ms_s[0], (16, 1)) + jnp.tile(ms_s[1], (16, 1))
        if D % 128:
            hn = jnp.concatenate([hn, jnp.zeros((128, npan * 128 - D), F32)], axis=-1)
        for p in range(npan):
            h_s[slot, p, c * 128:(c + 1) * 128, :] = hn[:, p * 128:(p + 1) * 128].astype(BF16)

    def get_h(slot):
        pans = [_unpack(h_i[slot, p]) for p in range(npan)]
        return jnp.concatenate(pans, axis=-1)[:, 0:D]

    def q_proj(i, slot, before=None):
        for j in range(nwq):
            if before is not None:
                before(j)
            q = jnp.dot(get_h(slot), wq_s[:, j * WQ_CHUNK:(j + 1) * WQ_CHUNK],
                        preferred_element_type=F32)
            for u in range(WQ_CHUNK // DH):
                q_s[j * (WQ_CHUNK // DH) + u, pl.ds(pl.multiple_of(i * RB, RB), RB), :] = (
                    q[:, u * DH:(u + 1) * DH] * qscale).astype(BF16)

    def fence():
        pl.semaphore_signal(sem_f, 1)
        pl.semaphore_wait(sem_f, 1)

    for cp in (c_copy, x_copy(0), moda_copy, wq_copy(0), wq_copy(1), x_copy(1), wq_copy(2), wq_copy(3),
               x_copy(2), wr_copy, modb_copy, k_copy, v_copy):
        cp.start()
        fence()
    c_copy.wait()
    x_copy(0).wait()
    cv = c_s[...].astype(F32)
    sc = _rb(cv * _rb(jax.nn.sigmoid(cv)))
    sc = jnp.broadcast_to(sc, (16, D)).astype(BF16)
    for c in range(RB // 128):
        xn_s[c] = normalise(0, c)
    moda_copy.wait()
    mod = _rb(jnp.dot(sc, wmod_s[:, 0:mod_a], preferred_element_type=F32))[0:8]
    ms_s[0] = _rb(1.0 + mod[:, D:2 * D])
    ms_s[1] = mod[:, 0:D]
    fence()
    for c in range(RB // 128):
        put_h(0, c, xn_s[c])
        fence()

    def first_block(j):
        for g in range(len(WQ_GROUPS)):
            if j == g_lo[g]:
                wq_copy(g).wait()
                if g == 2:
                    x_copy(1).wait()
        c = j - (nwq - RB // 128)
        if c >= 0:
            put_h(1, c, normalise(1, c))

    q_proj(0, 0, first_block)
    x_copy(2).wait()

    def p1_body(i, carry):
        def mid(j):
            if j % 2:
                c = j // 2
                put_h((i + 1) & 1, c, normalise(i + 1, c))

        q_proj(i, i & 1, mid)
        return carry

    lax.fori_loop(1, nrb - 1, p1_body, 0)

    wr_copy.wait()
    modb_copy.wait()
    k_copy.wait()
    v_copy.wait()
    for cp in late_copies:
        cp.start()
    mod2 = _rb(jnp.dot(sc, wmod_s[:, mod_a:6 * D], preferred_element_type=F32))[0:8]
    gb = mod2[:, 3 * D:4 * D]
    for n, row in enumerate((mod2[:, 0:D], mod2[:, D:2 * D], _rb(1.0 + mod2[:, 2 * D:3 * D]), gb,
                             wr_s[...].astype(F32).reshape(1, D))):
        col_s[n] = jnp.broadcast_to(row[0:1], (128, D)).T
    q_proj(nrb - 1, (nrb - 1) & 1)

    nbh = S // BQ
    nu = rep * nbh
    half = BQ // 2
    assert nu % 2 == 0

    def finish_max(slot):
        m = jnp.max(m_s[slot], axis=-1, keepdims=True)
        m_s[slot] = jnp.broadcast_to(m, (BQ, 128))

    def qk(h, u, defer):
        slot = u % 2
        q = _unpack(q_i[h * rep + u // nbh, (u % nbh) * half:(u % nbh + 1) * half, :])
        s = lax.dot_general(q, _unpack(k_i[h]), NT_DIMS, preferred_element_type=F32)
        s_s[slot] = s
        m_s[slot] = _fold(s, jnp.maximum)
        if not defer:
            finish_max(slot)

    def pv(h, u):
        slot = u % 2
        p = jnp.exp2(s_s[slot] - jnp.tile(m_s[slot], (1, S // 128)))
        l = jnp.sum(_fold(p, jnp.add), axis=-1, keepdims=True)
        acc = jnp.dot(p.astype(BF16), _unpack(v_i[h]), preferred_element_type=F32)
        inv = pl.reciprocal(l, approx=True)
        inv = inv * (2.0 - l * inv)
        o_s[h * rep + u // nbh, (u % nbh) * BQ:(u % nbh + 1) * BQ, :] = (acc * inv).astype(BF16)

    def p2_head(h, last):
        finish_max(1)
        for u in range(nu):
            pv(h, u)
            if u + 2 < nu:
                qk(h, u + 2, False)
            elif not last:
                qk(h + 1, u + 2 - nu, u == nu - 1)

    qk(0, 0, False)
    qk(0, 1, True)

    def p2_body(h, carry):
        p2_head(h, False)
        return carry

    lax.fori_loop(0, HKV - 1, p2_body, 0)
    for cp in late_copies:
        cp.wait()
    for j in range(F // 128):
        wdt_s[j * 128:(j + 1) * 128, :] = wd_s[:, j * 128:(j + 1) * 128].T
    p2_head(HKV - 1, True)

    def o_proj(t0):
        ob = jnp.concatenate(
            [_unpack(o_i[h, t0 // 2:t0 // 2 + 64, :]) for h in range(HQ)], axis=-1)
        wt = jnp.concatenate([_unpack(wo_i[h]) for h in range(HQ)], axis=-1)
        return lax.dot_general(wt, ob, NT_DIMS, preferred_element_type=F32)

    def resid_norm(t0, a):
        cols = pl.ds(t0, 128)
        x1 = _rb(x_s[:, cols].astype(F32) + col_s[0] * a)
        mean = jnp.sum(x1, axis=0, keepdims=True) * (1.0 / D)
        xc = x1 - mean
        var = jnp.sum(xc * xc, axis=0, keepdims=True) * (1.0 / D)
        std = _rb(jnp.sqrt(_rb(_rb(var) + LN_EPS_BF16)))
        hn = _rb(_rb(x1 - _rb(mean)) / std)
        h2 = _rb(_rb(hn * col_s[2]) + col_s[1])
        h2r_s[cols, :] = h2.astype(BF16).T
        x_s[:, cols] = (x1 + col_s[3] * h2).astype(BF16)
        out_copy(t0 // 128).start()
        rb = pltpu.bitcast(_rb(jnp.sum(h2 * col_s[4], axis=0, keepdims=True)), I32)
        tok = t0 + lax.broadcasted_iota(I32, (1, 128), 1)
        key = pltpu.bitcast(rb | jnp.where(rb >= 0, (S - 1) - tok, tok), F32)
        return jnp.where(sub == 0, key, -jnp.inf)

    sub = lax.broadcasted_iota(I32, (8, 128), 0)

    def max_all(a):
        m = jnp.max(jnp.max(a, axis=0, keepdims=True), axis=1, keepdims=True)
        return jnp.broadcast_to(m, (8, 128))

    def merge_top(top, kb):
        out = top
        for j in range(TOPC):
            m = max_all(jnp.maximum(top, kb))
            top = jnp.where(top == m, -jnp.inf, top)
            kb = jnp.where(kb == m, -jnp.inf, kb)
            out = jnp.where(sub == j, m, out)
        return out

    assert TOPC == 8 and S - 128 >= TOPC
    top = jnp.full((8, 128), -jnp.inf, F32)
    a = o_proj(0)
    for t0 in range(0, S - 128, 128):
        a_next = o_proj(t0 + 128)
        top = merge_top(top, resid_norm(t0, a))
        a = a_next
    kb = resid_norm(S - 128, a)

    def more(state):
        top, kb, best = state
        return jnp.max(jnp.where(best > jnp.min(top, axis=0, keepdims=True), 1, 0)) > 0

    def insert(state):
        top, kb, best = state
        top = jnp.where(top == jnp.min(top, axis=0, keepdims=True), best, top)
        kb = jnp.where(kb == best, -jnp.inf, kb)
        return top, kb, max_all(kb)

    top, _, _ = lax.while_loop(more, insert, (top, kb, max_all(kb)))

    def token_row(ref, idx):
        word = ref[pl.ds(lax.shift_right_logical(idx, 1), 1), :]
        bits = jnp.where((idx & 1) == 0, word << 16, word & jnp.int32(-65536))
        return pltpu.bitcast(jnp.broadcast_to(bits, (8, D)), F32)

    sub_d = lax.broadcasted_iota(I32, (8, D), 0)
    xsel = jnp.zeros((8, D), F32)
    top_bits = pltpu.bitcast(top, I32)
    low = top_bits & (S - 1)
    tok = jnp.where(top_bits >= 0, (S - 1) - low, low)
    idxs = []
    for j in range(TOPC):
        idx = tok[j, 0]
        idxs.append(idx)
        xsel = jnp.where(sub_d == j, token_row(h2r_s.bitcast(I32), idx), xsel)

    rsel = pltpu.bitcast(top_bits & jnp.int32(-65536), F32)[:, 0:1]
    xs = jnp.concatenate([xsel, xsel], axis=0).astype(BF16)
    g = _rb(jnp.dot(xs, wg_s[...], preferred_element_type=F32)[0:8])
    up = _rb(jnp.dot(xs, wu_s[...], preferred_element_type=F32)[0:8])
    act = _rb(_rb(g * _rb(jax.nn.sigmoid(g))) * up)
    act = jnp.concatenate([act, act], axis=0).astype(BF16)
    y = _rb(jnp.dot(act, wdt_s[...], preferred_element_type=F32)[0:8])
    y = _rb(y * _rb(jax.nn.sigmoid(rsel)))
    upd = gb * (_rb(xsel + y) - xsel)

    updt = jnp.concatenate([upd, jnp.zeros((8, D), F32)], axis=0).astype(BF16).T
    row16 = lax.broadcasted_iota(I32, (16, 128), 0)
    lane16 = lax.broadcasted_iota(I32, (16, 128), 1)
    idx_rows = jnp.full((16, 128), -1, I32)
    for j in range(TOPC):
        idx_rows = jnp.where(row16 == j, idxs[j], idx_rows)
    tiles = [lax.shift_right_logical(idx, 7) for idx in idxs]

    def tile_copy(j):
        cols = pl.ds(pl.multiple_of(tiles[j] * 128, 128), 128)
        return pltpu.make_async_copy(patch_s.at[j], o_hbm.at[:, cols], sem_p)

    def first_in_tile(j):
        return functools.reduce(jnp.logical_and, [tiles[j] != tiles[i] for i in range(j)], True)

    for t in range(S // 128):
        out_copy(t).wait()
    for j in range(TOPC):
        onehot = (idx_rows - tiles[j] * 128 == lane16).astype(BF16)
        moved = jnp.dot(updt, onehot, preferred_element_type=F32)
        old = x_s[:, pl.ds(pl.multiple_of(tiles[j] * 128, 128), 128)].astype(F32)
        patch_s[j] = (old + moved).astype(BF16)

        @pl.when(first_in_tile(j))
        def _():
            tile_copy(j).start()

    for j in range(TOPC):
        @pl.when(first_in_tile(j))
        def _():
            tile_copy(j).wait()


@jax.jit
def pallas_adaLN_cond__gqa_block_cached__moe_arch_mod__prompt_kernel(
    A_x: jax.Array,
    A_k_cache: jax.Array,
    A_v_cache: jax.Array,
    A_wq: jax.Array,
    A_wo: jax.Array,
    B_x: jax.Array,
    B_w_r: jax.Array,
    B_w_gate: jax.Array,
    B_w_up: jax.Array,
    B_w_down: jax.Array,
    c: jax.Array,
    w_mod: jax.Array,
):
    del B_x
    B, S, D = A_x.shape
    _, HKV, SK, DH = A_k_cache.shape
    HQ = A_wq.shape[1] // DH
    F = B_w_gate.shape[1]
    assert B == 1 and SK == S and DH == 128 and S % 1024 == 0 and S <= 65536

    vm = pltpu.VMEM
    dma = pltpu.SemaphoreType.DMA
    hbm = pl.BlockSpec(memory_space=pl.ANY)
    out = pl.pallas_call(
        functools.partial(_kernel, S=S, D=D, HQ=HQ, HKV=HKV, DH=DH, F=F),
        out_shape=jax.ShapeDtypeStruct((D, S), BF16),
        in_specs=[hbm] * 11,
        out_specs=hbm,
        scratch_shapes=[
            vm((D, S), BF16),
            vm((HKV, S, DH), BF16),
            vm((HKV, S, DH), BF16),
            vm((D, HQ * DH), BF16),
            vm((HQ, D, DH), BF16),
            vm((D, F), BF16),
            vm((D, F), BF16),
            vm((D, F), BF16),
            vm((D, 6 * D), BF16),
            vm((HQ, S, DH), BF16),
            vm((HQ, S, DH), BF16),
            vm((2, BQ, S), F32),
            vm((2, BQ, 128), F32),
            vm((2, -(-D // 128), RB, 128), BF16),
            vm((RB // 128, 128, D), F32),
            vm((2, 8, D), F32),
            vm((5, D, 128), F32),
            vm((S, D), BF16),
            vm((F, D), BF16),
            vm((TOPC, D, 128), BF16),
            vm((1, D), BF16),
            vm((D,), BF16),
            dma((3,)), dma((len(WQ_GROUPS),)), dma((6,)), dma, dma, dma,
            pltpu.SemaphoreType.REGULAR,
        ],
        compiler_params=pltpu.CompilerParams(
            vmem_limit_bytes=118 * 1024 * 1024,
            flags={"XLA_TPU_FORCE_LP_LLO_SCHEDULER": True},
        ),
        name="adaln_gqa_moe_block",
    )(c, B_w_r, A_x[0].T, A_k_cache[0], A_v_cache[0], A_wq, A_wo.T,
      B_w_gate, B_w_up, B_w_down.T, w_mod)
    return out.T[None]
```

```python
import functools

import jax
import jax.numpy as jnp
import jax.experimental.pallas as pl
import jax.experimental.pallas.tpu as pltpu
import numpy as np
from jax import lax

F32 = jnp.float32
BF16 = jnp.bfloat16
I32 = jnp.int32

NT_DIMS = (((1,), (1,)), ((), ()))
TOPC = 8
LN_EPS = 1e-5
LN_EPS_BF16 = float(np.asarray(LN_EPS, dtype=jnp.bfloat16))
LOG2E = 1.4426950408889634

RB = 512
BQ = 256
WQ_CHUNK = 512
WQ_GROUPS = (1, 2, 4, 1)


def _rb(a):
    return a.astype(BF16).astype(F32)


def _unpack(a):
    return pltpu.bitcast(a, BF16)


def _fold(a, op):
    out = a[:, :128]
    for j in range(1, a.shape[1] // 128):
        out = op(out, a[:, j * 128:(j + 1) * 128])
    return out


def _kernel(c_hbm, wr_hbm, x_hbm, k_hbm, v_hbm, wq_hbm, wo_hbm, wg_hbm, wu_hbm, wd_hbm,
            wmod_hbm, o_hbm,
            x_s, k_s, v_s, wq_s, wo_s, wg_s, wu_s, wd_s, wmod_s,
            q_s, o_s, s_s, m_s, h_s, xn_s, ms_s, col_s, h2r_s, wdt_s, patch_s,
            c_s, wr_s,
            sem_x, sem_wq, sem_w, sem_l, sem_o, sem_p, sem_f,
            *, S, D, HQ, HKV, DH, F):
    mod_a = 2 * D
    rep = HQ // HKV
    k_i = k_s.bitcast(I32)
    v_i = v_s.bitcast(I32)
    q_i = q_s.bitcast(I32)
    o_i = o_s.bitcast(I32)
    h_i = h_s.bitcast(I32)
    wo_i = wo_s.bitcast(I32)

    nrb = S // RB
    nwq = HQ * DH // WQ_CHUNK
    assert sum(WQ_GROUPS) == nwq and nrb >= 3 and nwq == 2 * (RB // 128)
    g_lo = np.cumsum((0,) + WQ_GROUPS)

    def x_copy(g):
        cols = pl.ds(g * RB, RB if g < 2 else S - 2 * RB)
        return pltpu.make_async_copy(x_hbm.at[:, cols], x_s.at[:, cols], sem_x.at[g])

    def wq_copy(g):
        cols = pl.ds(int(g_lo[g]) * WQ_CHUNK, WQ_GROUPS[g] * WQ_CHUNK)
        return pltpu.make_async_copy(wq_hbm.at[:, cols], wq_s.at[:, cols], sem_wq.at[g])

    def out_copy(t):
        cols = pl.ds(pl.multiple_of(t * 128, 128), 128)
        return pltpu.make_async_copy(x_s.at[:, cols], o_hbm.at[:, cols], sem_o)

    moda_copy = pltpu.make_async_copy(
        wmod_hbm.at[:, pl.ds(0, mod_a)], wmod_s.at[:, pl.ds(0, mod_a)], sem_w.at[0])
    modb_copy = pltpu.make_async_copy(
        wmod_hbm.at[:, pl.ds(mod_a, 4 * D)], wmod_s.at[:, pl.ds(mod_a, 4 * D)], sem_w.at[1])
    c_copy = pltpu.make_async_copy(c_hbm, c_s, sem_w.at[4])
    wr_copy = pltpu.make_async_copy(wr_hbm, wr_s, sem_w.at[5])
    k_copy = pltpu.make_async_copy(k_hbm, k_s, sem_w.at[2])
    v_copy = pltpu.make_async_copy(v_hbm, v_s, sem_w.at[3])
    late_copies = [
        pltpu.make_async_copy(wg_hbm, wg_s, sem_l),
        pltpu.make_async_copy(wu_hbm, wu_s, sem_l),
        pltpu.make_async_copy(wd_hbm, wd_s, sem_l),
    ] + [
        pltpu.make_async_copy(wo_hbm.at[:, pl.ds(h * DH, DH)], wo_s.at[h], sem_l)
        for h in range(HQ)
    ]

    npan = -(-D // 128)
    qscale = (DH ** -0.5) * LOG2E

    def normalise(i, c):
        cols = pl.ds(pl.multiple_of(i * RB + c * 128, 128), 128)
        xv = x_s[:, cols].T.astype(F32)
        mean = jnp.sum(xv, axis=-1, keepdims=True) * (1.0 / D)
        xc = xv - mean
        var = jnp.sum(xc * xc, axis=-1, keepdims=True) * (1.0 / D)
        return xc * lax.rsqrt(var + LN_EPS)

    def put_h(slot, c, xn):
        hn = xn * jnp.tile(ms_s[0], (16, 1)) + jnp.tile(ms_s[1], (16, 1))
        if D % 128:
            hn = jnp.concatenate([hn, jnp.zeros((128, npan * 128 - D), F32)], axis=-1)
        for p in range(npan):
            h_s[slot, p, c * 128:(c + 1) * 128, :] = hn[:, p * 128:(p + 1) * 128].astype(BF16)

    def get_h(slot):
        pans = [_unpack(h_i[slot, p]) for p in range(npan)]
        return jnp.concatenate(pans, axis=-1)[:, 0:D]

    def q_proj(i, slot, before=None):
        for j in range(nwq):
            if before is not None:
                before(j)
            q = jnp.dot(get_h(slot), wq_s[:, j * WQ_CHUNK:(j + 1) * WQ_CHUNK],
                        preferred_element_type=F32)
            for u in range(WQ_CHUNK // DH):
                q_s[j * (WQ_CHUNK // DH) + u, pl.ds(pl.multiple_of(i * RB, RB), RB), :] = (
                    q[:, u * DH:(u + 1) * DH] * qscale).astype(BF16)

    def fence():
        pl.semaphore_signal(sem_f, 1)
        pl.semaphore_wait(sem_f, 1)

    for cp in (c_copy, x_copy(0), moda_copy, wq_copy(0), wq_copy(1), x_copy(1), wq_copy(2), wq_copy(3),
               x_copy(2), wr_copy, modb_copy, k_copy, v_copy):
        cp.start()
        fence()
    c_copy.wait()
    x_copy(0).wait()
    cv = c_s[...].astype(F32)
    sc = _rb(cv * _rb(jax.nn.sigmoid(cv)))
    sc = jnp.broadcast_to(sc, (16, D)).astype(BF16)
    for c in range(RB // 128):
        xn_s[c] = normalise(0, c)
    moda_copy.wait()
    mod = _rb(jnp.dot(sc, wmod_s[:, 0:mod_a], preferred_element_type=F32))[0:8]
    ms_s[0] = _rb(1.0 + mod[:, D:2 * D])
    ms_s[1] = mod[:, 0:D]
    fence()
    for c in range(RB // 128):
        put_h(0, c, xn_s[c])
        fence()

    def first_block(j):
        for g in range(len(WQ_GROUPS)):
            if j == g_lo[g]:
                wq_copy(g).wait()
                if g == 2:
                    x_copy(1).wait()
        c = j - (nwq - RB // 128)
        if c >= 0:
            put_h(1, c, normalise(1, c))

    q_proj(0, 0, first_block)
    x_copy(2).wait()

    def p1_body(i, carry):
        def mid(j):
            if j % 2:
                c = j // 2
                put_h((i + 1) & 1, c, normalise(i + 1, c))

        q_proj(i, i & 1, mid)
        return carry

    lax.fori_loop(1, nrb - 1, p1_body, 0)

    wr_copy.wait()
    modb_copy.wait()
    k_copy.wait()
    v_copy.wait()
    for cp in late_copies:
        cp.start()
    mod2 = _rb(jnp.dot(sc, wmod_s[:, mod_a:6 * D], preferred_element_type=F32))[0:8]
    gb = mod2[:, 3 * D:4 * D]
    for n, row in enumerate((mod2[:, 0:D], mod2[:, D:2 * D], _rb(1.0 + mod2[:, 2 * D:3 * D]), gb,
                             wr_s[...].astype(F32).reshape(1, D))):
        col_s[n] = jnp.broadcast_to(row[0:1], (128, D)).T
    q_proj(nrb - 1, (nrb - 1) & 1)

    nbh = S // BQ
    nu = rep * nbh
    half = BQ // 2
    assert nu % 2 == 0

    def finish_max(slot):
        m = jnp.max(m_s[slot], axis=-1, keepdims=True)
        m_s[slot] = jnp.broadcast_to(m, (BQ, 128))

    def qk(h, u, defer):
        slot = u % 2
        q = _unpack(q_i[h * rep + u // nbh, (u % nbh) * half:(u % nbh + 1) * half, :])
        s = lax.dot_general(q, _unpack(k_i[h]), NT_DIMS, preferred_element_type=F32)
        s_s[slot] = s
        m_s[slot] = _fold(s, jnp.maximum)
        if not defer:
            finish_max(slot)

    def pv(h, u):
        slot = u % 2
        p = jnp.exp2(s_s[slot] - jnp.tile(m_s[slot], (1, S // 128)))
        l = jnp.sum(_fold(p, jnp.add), axis=-1, keepdims=True)
        acc = jnp.dot(p.astype(BF16), _unpack(v_i[h]), preferred_element_type=F32)
        inv = pl.reciprocal(l, approx=True)
        inv = inv * (2.0 - l * inv)
        o_s[h * rep + u // nbh, (u % nbh) * BQ:(u % nbh + 1) * BQ, :] = (acc * inv).astype(BF16)

    def p2_head(h, last):
        finish_max(1)
        for u in range(nu):
            pv(h, u)
            if u + 2 < nu:
                qk(h, u + 2, False)
            elif not last:
                qk(h + 1, u + 2 - nu, u == nu - 1)

    qk(0, 0, False)
    qk(0, 1, True)

    def p2_body(h, carry):
        p2_head(h, False)
        return carry

    lax.fori_loop(0, HKV - 1, p2_body, 0)
    for cp in late_copies:
        cp.wait()
    for j in range(F // 128):
        wdt_s[j * 128:(j + 1) * 128, :] = wd_s[:, j * 128:(j + 1) * 128].T
    p2_head(HKV - 1, True)

    def o_proj(t0):
        ob = jnp.concatenate(
            [_unpack(o_i[h, t0 // 2:t0 // 2 + 64, :]) for h in range(HQ)], axis=-1)
        wt = jnp.concatenate([_unpack(wo_i[h]) for h in range(HQ)], axis=-1)
        return lax.dot_general(wt, ob, NT_DIMS, preferred_element_type=F32)

    def resid_norm(t0, a):
        cols = pl.ds(t0, 128)
        x1 = _rb(x_s[:, cols].astype(F32) + col_s[0] * a)
        mean = jnp.sum(x1, axis=0, keepdims=True) * (1.0 / D)
        xc = x1 - mean
        var = jnp.sum(xc * xc, axis=0, keepdims=True) * (1.0 / D)
        std = _rb(jnp.sqrt(_rb(_rb(var) + LN_EPS_BF16)))
        hn = _rb(_rb(x1 - _rb(mean)) / std)
        h2 = _rb(_rb(hn * col_s[2]) + col_s[1])
        h2r_s[cols, :] = h2.astype(BF16).T
        x_s[:, cols] = (x1 + col_s[3] * h2).astype(BF16)
        out_copy(t0 // 128).start()
        rb = pltpu.bitcast(_rb(jnp.sum(h2 * col_s[4], axis=0, keepdims=True)), I32)
        tok = t0 + lax.broadcasted_iota(I32, (1, 128), 1)
        key = pltpu.bitcast(rb | jnp.where(rb >= 0, (S - 1) - tok, tok), F32)
        return jnp.where(sub == 0, key, -jnp.inf)

    sub = lax.broadcasted_iota(I32, (8, 128), 0)

    def max_all(a):
        m = jnp.max(jnp.max(a, axis=0, keepdims=True), axis=1, keepdims=True)
        return jnp.broadcast_to(m, (8, 128))

    def merge_top(top, kb):
        out = top
        for j in range(TOPC):
            m = max_all(jnp.maximum(top, kb))
            top = jnp.where(top == m, -jnp.inf, top)
            kb = jnp.where(kb == m, -jnp.inf, kb)
            out = jnp.where(sub == j, m, out)
        return out

    assert TOPC == 8 and S - 128 >= TOPC
    top = jnp.full((8, 128), -jnp.inf, F32)
    a = o_proj(0)
    for t0 in range(0, S - 128, 128):
        a_next = o_proj(t0 + 128)
        top = merge_top(top, resid_norm(t0, a))
        a = a_next
    kb = resid_norm(S - 128, a)

    def more(state):
        top, kb, best = state
        return jnp.max(jnp.where(best > jnp.min(top, axis=0, keepdims=True), 1, 0)) > 0

    def insert(state):
        top, kb, best = state
        top = jnp.where(top == jnp.min(top, axis=0, keepdims=True), best, top)
        kb = jnp.where(kb == best, -jnp.inf, kb)
        return top, kb, max_all(kb)

    top, _, _ = lax.while_loop(more, insert, (top, kb, max_all(kb)))

    def token_row(ref, idx):
        word = ref[pl.ds(lax.shift_right_logical(idx, 1), 1), :]
        bits = jnp.where((idx & 1) == 0, word << 16, word & jnp.int32(-65536))
        return pltpu.bitcast(jnp.broadcast_to(bits, (8, D)), F32)

    sub_d = lax.broadcasted_iota(I32, (8, D), 0)
    xsel = jnp.zeros((8, D), F32)
    top_bits = pltpu.bitcast(top, I32)
    low = top_bits & (S - 1)
    tok = jnp.where(top_bits >= 0, (S - 1) - low, low)
    idxs = []
    for j in range(TOPC):
        idx = tok[j, 0]
        idxs.append(idx)
        xsel = jnp.where(sub_d == j, token_row(h2r_s.bitcast(I32), idx), xsel)

    rsel = pltpu.bitcast(top_bits & jnp.int32(-65536), F32)[:, 0:1]
    xs = jnp.concatenate([xsel, xsel], axis=0).astype(BF16)
    for t in range(S // 128):
        out_copy(t).wait()
    g = _rb(jnp.dot(xs, wg_s[...], preferred_element_type=F32)[0:8])
    up = _rb(jnp.dot(xs, wu_s[...], preferred_element_type=F32)[0:8])
    act = _rb(_rb(g * _rb(jax.nn.sigmoid(g))) * up)
    act = jnp.concatenate([act, act], axis=0).astype(BF16)
    y = _rb(jnp.dot(act, wdt_s[...], preferred_element_type=F32)[0:8])
    y = _rb(y * _rb(jax.nn.sigmoid(rsel)))
    upd = gb * (_rb(xsel + y) - xsel)

    updt = jnp.concatenate([upd, jnp.zeros((8, D), F32)], axis=0).astype(BF16).T
    row16 = lax.broadcasted_iota(I32, (16, 128), 0)
    lane16 = lax.broadcasted_iota(I32, (16, 128), 1)
    idx_rows = jnp.full((16, 128), -1, I32)
    for j in range(TOPC):
        idx_rows = jnp.where(row16 == j, idxs[j], idx_rows)
    tiles = [lax.shift_right_logical(idx, 7) for idx in idxs]

    def tile_copy(j):
        cols = pl.ds(pl.multiple_of(tiles[j] * 128, 128), 128)
        return pltpu.make_async_copy(patch_s.at[j], o_hbm.at[:, cols], sem_p)

    def first_in_tile(j):
        return functools.reduce(jnp.logical_and, [tiles[j] != tiles[i] for i in range(j)], True)

    for j in range(TOPC):
        onehot = (idx_rows - tiles[j] * 128 == lane16).astype(BF16)
        for part in range(3):
            rows = slice(part * D // 3, (part + 1) * D // 3)
            moved = jnp.dot(updt[rows], onehot, preferred_element_type=F32)
            old = x_s[rows, pl.ds(pl.multiple_of(tiles[j] * 128, 128), 128)].astype(F32)
            patch_s[j, rows] = (old + moved).astype(BF16)

        @pl.when(first_in_tile(j))
        def _():
            tile_copy(j).start()

    for j in range(TOPC):
        @pl.when(first_in_tile(j))
        def _():
            tile_copy(j).wait()


@jax.jit
def pallas_adaLN_cond__gqa_block_cached__moe_arch_mod__prompt_kernel(
    A_x: jax.Array,
    A_k_cache: jax.Array,
    A_v_cache: jax.Array,
    A_wq: jax.Array,
    A_wo: jax.Array,
    B_x: jax.Array,
    B_w_r: jax.Array,
    B_w_gate: jax.Array,
    B_w_up: jax.Array,
    B_w_down: jax.Array,
    c: jax.Array,
    w_mod: jax.Array,
):
    del B_x
    B, S, D = A_x.shape
    _, HKV, SK, DH = A_k_cache.shape
    HQ = A_wq.shape[1] // DH
    F = B_w_gate.shape[1]
    assert B == 1 and SK == S and DH == 128 and S % 1024 == 0 and S <= 65536 and S & (S - 1) == 0

    vm = pltpu.VMEM
    dma = pltpu.SemaphoreType.DMA
    hbm = pl.BlockSpec(memory_space=pl.ANY)
    out = pl.pallas_call(
        functools.partial(_kernel, S=S, D=D, HQ=HQ, HKV=HKV, DH=DH, F=F),
        out_shape=jax.ShapeDtypeStruct((D, S), BF16),
        in_specs=[hbm] * 11,
        out_specs=hbm,
        scratch_shapes=[
            vm((D, S), BF16),
            vm((HKV, S, DH), BF16),
            vm((HKV, S, DH), BF16),
            vm((D, HQ * DH), BF16),
            vm((HQ, D, DH), BF16),
            vm((D, F), BF16),
            vm((D, F), BF16),
            vm((D, F), BF16),
            vm((D, 6 * D), BF16),
            vm((HQ, S, DH), BF16),
            vm((HQ, S, DH), BF16),
            vm((2, BQ, S), F32),
            vm((2, BQ, 128), F32),
            vm((2, -(-D // 128), RB, 128), BF16),
            vm((RB // 128, 128, D), F32),
            vm((2, 8, D), F32),
            vm((5, D, 128), F32),
            vm((S, D), BF16),
            vm((F, D), BF16),
            vm((TOPC, D, 128), BF16),
            vm((1, D), BF16),
            vm((D,), BF16),
            dma((3,)), dma((len(WQ_GROUPS),)), dma((6,)), dma, dma, dma,
            pltpu.SemaphoreType.REGULAR,
        ],
        compiler_params=pltpu.CompilerParams(
            vmem_limit_bytes=118 * 1024 * 1024,
            flags={"XLA_TPU_FORCE_LP_LLO_SCHEDULER": True},
        ),
        name="adaln_gqa_moe_block",
    )(c, B_w_r, A_x[0].T, A_k_cache[0], A_v_cache[0], A_wq, A_wo.T,
      B_w_gate, B_w_up, B_w_down.T, w_mod)
    return out.T[None]
```
